```python
import jax
import jax.numpy as jnp

def _softmax(x, axis=-1):
    return jax.nn.softmax(x, axis=axis)

def _gelu(x):
    return jax.nn.gelu(x, approximate=True)

def _silu(x):
    return jax.nn.silu(x)

def _sigmoid(x):
    return jax.nn.sigmoid(x)

def _layernorm(x, axis=-1, eps=1e-05):
    m = jnp.mean(x, axis=axis, keepdims=True)
    v = jnp.var(x, axis=axis, keepdims=True)
    return (x - m) / jnp.sqrt(v + eps)

def _scatter_add(tgt, idx, src, axis=0):
    return tgt.at[idx].add(src)

def _segment_sum(src, seg, n):
    return jax.ops.segment_sum(src, seg, n)

class _Rng:

    def __init__(self, key):
        self._k = key

    def _next(self):
        self._k, sub = jax.random.split(self._k)
        return sub

    def normal(self, shape):
        return jax.random.normal(self._next(), shape, dtype=jnp.bfloat16)

    def randint(self, lo, hi, shape):
        return jax.random.randint(self._next(), shape, lo, hi, dtype=jnp.int32)

    def uniform(self, shape, lo=0.0, hi=1.0):
        return jax.random.uniform(self._next(), shape, jnp.bfloat16, lo, hi)

    def permutation(self, n):
        return jax.random.permutation(self._next(), n)
kernel_name = 'sequential_preLN__memory_aug_recurrent_mem_tr__mixer_s_mlp__prompt'

def setup_inputs():
    _rng = _Rng(jax.random.key(int.from_bytes(__import__("os").urandom(4), "little")))
    _w = lambda a: (lambda t: t.astype(jnp.bfloat16) if jnp.issubdtype(t.dtype, jnp.floating) else t)(jnp.asarray(a))

    def _A_setup():
        B, S, Dm = (1, 2048, 1024)
        H, Dh = (32, 128)
        M, seg = (8, 32)
        seg = min(seg, S)
        S = S // seg * seg
        return {'x': _w((lambda *s: _rng.normal(s) * 0.05)(B, S, Dm)), 'mem0': _w((lambda *s: _rng.normal(s) * 0.05)(B, M, Dm)), 'Wq': _w((lambda *s: _rng.normal(s) * 0.05)(Dm, H, Dh) * Dm ** (-0.5)), 'Wk': _w((lambda *s: _rng.normal(s) * 0.05)(Dm, H, Dh) * Dm ** (-0.5)), 'Wv': _w((lambda *s: _rng.normal(s) * 0.05)(Dm, H, Dh) * Dm ** (-0.5)), 'Wo': _w((lambda *s: _rng.normal(s) * 0.05)(H, Dh, Dm) * (H * Dh) ** (-0.5)), 'seg_len': seg}
    _A_in = _A_setup()

    def _B_setup():
        B, S, D, F = (1, 2048, 1024, 3584)
        return {'x': _w((lambda *s: _rng.normal(s) * 0.05)(B, S, D)), 'w1': _w((lambda *s: _rng.normal(s) * 0.05)(D, D) * D ** (-0.5)), 'w2': _w((lambda *s: _rng.normal(s) * 0.05)(D, D) * D ** (-0.5)), 'w3': _w((lambda *s: _rng.normal(s) * 0.05)(D, F) * D ** (-0.5)), 'w4': _w((lambda *s: _rng.normal(s) * 0.05)(F, D) * F ** (-0.5))}
    _B_in = _B_setup()
    return {'A_x': _A_in['x'], 'A_mem0': _A_in['mem0'], 'A_Wq': _A_in['Wq'], 'A_Wk': _A_in['Wk'], 'A_Wv': _A_in['Wv'], 'A_Wo': _A_in['Wo'], 'A_seg_len': _A_in['seg_len'], 'B_x': _B_in['x'], 'B_w1': _B_in['w1'], 'B_w2': _B_in['w2'], 'B_w3': _B_in['w3'], 'B_w4': _B_in['w4']}

def reference(A_x, A_mem0, A_Wq, A_Wk, A_Wv, A_Wo, A_seg_len, B_x, B_w1, B_w2, B_w3, B_w4):

    def _A_ref(x, mem0, Wq, Wk, Wv, Wo, seg_len):
        B, S, Dm = x.shape
        H, Dh = (Wq.shape[1], Wq.shape[2])
        M = mem0.shape[1]
        scale = Dh ** (-0.5)
        n_seg = S // seg_len
        L = M + seg_len
        idx = jnp.arange(L)
        mask = (idx[:, None] < M) | (idx[:, None] >= idx[None, :])
        mem = mem0
        outs = []
        for s in range(n_seg):
            xs = x[:, s * seg_len:(s + 1) * seg_len, :].copy()
            h = jnp.concatenate([mem, xs], axis=1)
            q = jnp.einsum('btd,dhe->bhte', h, Wq)
            k = jnp.einsum('btd,dhe->bhte', h, Wk)
            v = jnp.einsum('btd,dhe->bhte', h, Wv)
            scores = jnp.einsum('bhqe,bhke->bhqk', q, k) * scale
            scores = jnp.where(mask[None, None], scores, -1000000000.0)
            p = _softmax(scores, axis=-1)
            o = jnp.einsum('bhqk,bhke->bhqe', p, v)
            o = jnp.einsum('bhte,hed->btd', o, Wo)
            mem = o[:, :M, :].copy()
            outs.append(o[:, M:, :])
        return jnp.concatenate(outs, axis=1)

    def _B_ref(x, w1, w2, w3, w4):
        B, S, D = x.shape
        h = _gelu(_layernorm(x, axis=-1) @ w1)
        c = D // 4
        g0 = jnp.pad(h[:, :, 0 * c:1 * c], ((0, 0), (1, 0), (0, 0)))[:, :S, :]
        g1 = jnp.pad(h[:, :, 1 * c:2 * c], ((0, 0), (0, 1), (0, 0)))[:, 1:, :]
        g2 = jnp.pad(h[:, :, 2 * c:3 * c], ((0, 0), (2, 0), (0, 0)))[:, :S, :]
        g3 = jnp.pad(h[:, :, 3 * c:], ((0, 0), (0, 2), (0, 0)))[:, 2:, :]
        hs = jnp.concatenate([g0, g1, g2, g3], axis=-1) @ w2
        x1 = x + hs
        h2 = _gelu(_layernorm(x1, axis=-1) @ w3) @ w4
        return x1 + h2
    x = A_x
    h = x + _A_ref(_layernorm(x, axis=-1), A_mem0, A_Wq, A_Wk, A_Wv, A_Wo, A_seg_len)
    h2 = h + _B_ref(_layernorm(h, axis=-1), B_w1, B_w2, B_w3, B_w4)
    return h2
```

```python
import jax
import jax.numpy as jnp
from jax import lax
import jax.experimental.pallas as pl
import jax.experimental.pallas.tpu as pltpu

S = 2048
D = 1024
H = 32
DH = 128
MEM = 8
SEG = 32
F = 3584
NSEG = S // SEG
L = MEM + SEG
TOK = 24
P0 = S - TOK * NSEG
RING = 576
C4 = D // 4
HALO = 8
RB = 256
FC = 512
EPS = 1e-5
NEG = -1000000000.0

bf16 = jnp.bfloat16
f32 = jnp.float32
u32 = jnp.uint32

LAG_QK = 1
LAG_PV = 4
LAG_WO = 11
WO_GROUP = 1


def _ln(x):
    m = jnp.mean(x, axis=-1, keepdims=True)
    d = x - m
    v = jnp.mean(d * d, axis=-1, keepdims=True)
    return d * lax.rsqrt(v + EPS)


def _gelu(x):
    return jax.nn.gelu(x, approximate=True)


def _pack(x):
    return pltpu.bitcast(x.astype(bf16), u32)


def _unpack(x):
    return pltpu.bitcast(x, bf16)


def _dot(a, b):
    return jnp.dot(a, b, preferred_element_type=f32)


def _kernel(x_hbm, mem0_ref, wq_hbm, wk_hbm, wv_hbm, wo_hbm, w1_hbm, w2_hbm,
            w3_hbm, w4_hbm, out_hbm,
            wq_s, wk_s, wv_s, wo_s, stg0, stg1, stg2, xs, hbuf, xg, lhs0, ubuf,
            w1b, w2b, w3b, w4b, yall, t0, t1, acc, sems, *rings):
    w_hbm = (wq_hbm, wk_hbm, wv_hbm)
    w_s = (wq_s, wk_s, wv_s)
    stg = (stg0, stg1, stg2)
    ring = [[rings[m * 8 + h % 8].at[h // 8] for h in range(H)] for m in range(3)]
    q_r, k_r, v_r = ring

    SEM_X, SEM_W, SEM_WO, SEM_W1, SEM_W2, SEM_W3, SEM_W4, SEM_OUT = (
        0, 4, 16, 21, 25, 26, 27, 28)

    def x_copy(i):
        rows = pl.ds(i * 512, 512)
        return pltpu.make_async_copy(x_hbm.at[rows], xs.at[rows], sems.at[SEM_X + i])

    def w_copy(c):
        g, m = divmod(c, 3)
        return pltpu.make_async_copy(
            w_hbm[m].at[:, pl.ds(8 * g, 8), :], stg[m], sems.at[SEM_W + c])

    def wo_copies(q):
        if q < 3:
            rows = pl.ds(q * 1024, 1024)
            return [pltpu.make_async_copy(wo_hbm.at[rows], w4b.at[rows],
                                          sems.at[SEM_WO + q])]
        return [pltpu.make_async_copy(wo_hbm.at[pl.ds(3072, 512)],
                                      w4b.at[pl.ds(3072, 512)], sems.at[SEM_WO + 3]),
                pltpu.make_async_copy(wo_hbm.at[pl.ds(3584, 512)],
                                      w2b.at[pl.ds(0, 512)], sems.at[SEM_WO + 4])]

    def w1_copy(i):
        return pltpu.make_async_copy(
            w1_hbm.at[:, pl.ds(i * C4, C4)], w1b.at[i], sems.at[SEM_W1 + i])

    w2_copy = pltpu.make_async_copy(w2_hbm, w2b, sems.at[SEM_W2])
    w3_copy = pltpu.make_async_copy(w3_hbm, w3b, sems.at[SEM_W3])
    w4_copy = pltpu.make_async_copy(w4_hbm, w4b, sems.at[SEM_W4])

    def out_copy(i):
        rows = pl.ds(pl.multiple_of(i * RB, RB), RB)
        return pltpu.make_async_copy(xs.at[rows], out_hbm.at[rows], sems.at[SEM_OUT + i])

    def norm_rows(r0, n, to_lhs0):
        xv = xs[pl.ds(r0, n), :].astype(f32)
        hbuf[pl.ds(r0, n), :] = xv
        xn = _ln(xv)
        if to_lhs0:
            lhs0[pl.ds(r0 // 2, n // 2), :] = _pack(xn)
        else:
            for c in range(4):
                xg[c, pl.ds(HALO + r0, n), :] = xn[:, c * C4:(c + 1) * C4]

    def relayout(c):
        g, m = divmod(c, 3)
        for blk in range(8):
            w = stg[m][pl.ds(blk * 128, 128), :, :]
            wt = jnp.transpose(w, (1, 0, 2))
            w_s[m][pl.ds(8 * g, 8), pl.ds(blk * 64, 64), :] = pltpu.bitcast(wt, u32)

    def repack_wo(q):
        for blk in range(4):
            r0 = q * 1024 + blk * 256
            src = w4b if r0 < 3584 else w2b
            s0 = r0 if r0 < 3584 else r0 - 3584
            wo_s[pl.ds(r0 // 2, 128), :] = pltpu.bitcast(src[pl.ds(s0, 256), :], u32)

    def batch_proj(c):
        g, m = divmod(c, 3)
        lhs = _unpack(lhs0[...])
        for h in range(8 * g, 8 * g + 8):
            ring[m][h][pl.ds(0, P0), :] = _dot(lhs, _unpack(w_s[m][h]))

    x_copy(0).start()
    w_copy(0).start()
    zero = jnp.zeros((HALO, C4), f32)
    for c in range(4):
        xg[c, pl.ds(0, HALO), :] = zero
        xg[c, pl.ds(HALO + S, HALO), :] = zero
    x_copy(0).wait()
    w_copy(1).start()
    w_copy(2).start()
    norm_rows(0, 256, True)
    norm_rows(256, 256, True)
    x_copy(1).start()
    w_copy(0).wait()
    relayout(0)
    w_copy(3).start()
    for c in range(12):
        if c + 1 < 12:
            w_copy(c + 1).wait()
            relayout(c + 1)
            if c + 4 < 12:
                w_copy(c + 4).start()
        if c in (0, 1):
            x_copy(c + 2).start()
        if c in (0, 4, 8):
            x_copy(1 + c // 4).wait()
        norm_rows(P0 + c * 128, 128, False)
        if 1 <= c <= 4:
            for cp in wo_copies(c - 1):
                cp.start()
        if c in (4, 6, 8, 10):
            q = (c - 4) // 2
            for cp in wo_copies(q):
                cp.wait()
            repack_wo(q)
        if c == 5:
            for i in range(4):
                w1_copy(i).start()
        if c == 7:
            w3_copy.start()
        if c == 11:
            w4_copy.start()
            w2_copy.start()
        batch_proj(c)
    for i in range(4):
        w1_copy(i).wait()

    def wrap(r):
        return jnp.where(r >= RING, r - RING, r)

    def step(s, carry):
        mem, rp, ra, rw = carry
        ri = lax.broadcasted_iota(jnp.int32, (L, L), 0)
        ci = lax.broadcasted_iota(jnp.int32, (L, L), 1)
        mask = (ri < MEM) | (ri >= ci)

        t_tok = pl.multiple_of(HALO + P0 + TOK * s, 8)
        tok = jnp.concatenate([xg[c, pl.ds(t_tok, TOK), :] for c in range(4)], axis=1)
        lhs = jnp.concatenate([mem, tok], axis=0).astype(bf16)
        rps = [pl.multiple_of(wrap(rp + 8 * i), 8) for i in range(3)]
        ra_ = pl.multiple_of(ra, SEG)
        rw_ = pl.multiple_of(rw, 8)

        col = s & 3
        rb = pl.multiple_of(jnp.maximum((s >> 2) - 1, 0) * (4 * TOK), 8)
        ubuf[...] = _pack(_ln(_ln(hbuf[pl.ds(rb, 4 * TOK), :])))

        def filler(j):
            u = _unpack(ubuf[...])
            r = _dot(u, w1b[col, :, pl.ds(j * 128, 128)])
            xg[col, pl.ds(HALO + rb, 4 * TOK), pl.ds(j * 128, 128)] = _gelu(r)

        mem_qkv = {}
        scores = {}
        o_mem = {}
        total = [None]

        def qkv(h):
            res = []
            for m in range(3):
                r = _dot(lhs, _unpack(w_s[m][h]))
                for i in range(3):
                    ring[m][h][pl.ds(rps[i], 8), :] = r[8 + 8 * i:16 + 8 * i]
                res.append(r[:MEM])
            mem_qkv[h] = res

        def qk(h):
            qm, km, vm = mem_qkv.pop(h)
            qa = jnp.concatenate([qm, q_r[h][pl.ds(ra_, SEG), :]], axis=0).astype(bf16)
            ka = jnp.concatenate([km, k_r[h][pl.ds(ra_, SEG), :]], axis=0).astype(bf16)
            sc = lax.dot_general(qa, ka, (((1,), (1,)), ((), ())),
                                 preferred_element_type=f32)
            scores[h] = (sc, vm)

        def pv(h):
            sc, vm = scores.pop(h)
            va = jnp.concatenate([vm, v_r[h][pl.ds(ra_, SEG), :]], axis=0).astype(bf16)
            sc = jnp.where(mask, sc * (DH ** -0.5), NEG)
            mx = jnp.max(sc, axis=1, keepdims=True)
            e = jnp.exp(sc - mx)
            den = jnp.sum(e, axis=1, keepdims=True)
            inv = pl.reciprocal(den, approx=True)
            inv = inv * (2.0 - den * inv)
            o = _dot(e.astype(bf16), va) * inv
            q_r[h][pl.ds(ra_, SEG), :] = o[MEM:]
            o_mem[h] = o[:MEM]

        def wo(g):
            hs = range(g * WO_GROUP, (g + 1) * WO_GROUP)
            lo = jnp.concatenate(
                [jnp.concatenate([o_mem.pop(h), q_r[h][pl.ds(rw_, TOK), :]], axis=0)
                 for h in hs], axis=1).astype(bf16)
            w = _unpack(wo_s[pl.ds(g * WO_GROUP * 64, WO_GROUP * 64), :])
            r = _dot(lo, w)
            total[0] = r if total[0] is None else total[0] + r

        ng = H // WO_GROUP
        nxt = 0
        done_pv = 0
        t = 0
        while nxt < ng:
            if t < H:
                qkv(t)
            if 0 <= t - LAG_QK < H:
                qk(t - LAG_QK)
            if t == H + LAG_QK:
                filler(0)
            if 0 <= t - LAG_PV < H:
                pv(t - LAG_PV)
                done_pv = t - LAG_PV + 1
            while (nxt < ng and t >= (nxt + 1) * WO_GROUP - 1 + LAG_WO
                   and done_pv >= (nxt + 1) * WO_GROUP):
                wo(nxt)
                nxt += 1
            t += 1
        filler(1)

        a = total[0]
        hr = pl.multiple_of(TOK * s, 8)
        hbuf[pl.ds(hr, TOK), :] += a[MEM:]
        return a[:MEM], wrap(rp + TOK), wrap(ra + SEG), wrap(rw + TOK)

    lax.fori_loop(
        0, NSEG, step,
        (mem0_ref[...].astype(f32), jnp.int32(P0), jnp.int32(0), jnp.int32(0)))

    w2_copy.wait()
    w3_copy.wait()
    w4_copy.wait()

    def wo_batch(r0, n):
        rr = r0 % RING
        lo = jnp.concatenate(
            [q_r[h][pl.ds(rr, n), :].astype(bf16) for h in range(H)], axis=1)
        hbuf[pl.ds(r0, n), :] += _dot(lo, _unpack(wo_s[...]))

    def mixer_in(r0, n):
        u = _ln(_ln(hbuf[pl.ds(r0, n), :])).astype(bf16)
        for c in range(4):
            xg[c, pl.ds(HALO + r0, n), :] = _gelu(_dot(u, w1b[c]))

    def mixer_out(i):
        r0 = i * RB
        parts = []
        for c, off in enumerate((-1, 1, -2, 2)):
            win = xg[c, pl.ds(r0, RB + 2 * HALO), :]
            parts.append(win[HALO + off:HALO + off + RB])
        hs = _dot(jnp.concatenate(parts, axis=1).astype(bf16), w2b[...])
        hv = hbuf[pl.ds(r0, RB), :]
        x1 = _ln(hv) + hs
        yall[pl.ds(r0 // 2, RB // 2), :] = _pack(_ln(x1))
        hbuf[pl.ds(r0, RB), :] = hv + x1

    done = TOK * NSEG
    split = 3 * RING
    first = 4 * TOK * (NSEG // 4 - 1)
    wo_batch(done, split - done)
    wo_batch(split, S - split)
    mixer_out(0)
    mixer_in(first, split - first)
    mixer_out(1)
    mixer_in(split, S - split)
    for i in range(2, S // RB):
        mixer_out(i)

    ts = (t0, t1)
    nc = F // FC

    def mlp_block(i, carry):
        rows = pl.ds(pl.multiple_of(i * RB, RB), RB)

        def up(c):
            y = _unpack(yall[pl.ds(pl.multiple_of(i * (RB // 2), RB // 2), RB // 2), :])
            r = _dot(y, w3b[:, c * FC:(c + 1) * FC])
            ts[c % 2][...] = _pack(_gelu(r))

        def down(c):
            r = _dot(_unpack(ts[c % 2][...]), w4b[c * FC:(c + 1) * FC, :])
            if c == 0:
                acc[...] = hbuf[rows, :] + r
            elif c < nc - 1:
                acc[...] += r
            else:
                xs[rows, :] = (acc[...] + r).astype(bf16)

        up(0)
        for c in range(nc):
            if c + 1 < nc:
                up(c + 1)
            down(c)
        out_copy(i).start()
        return carry

    lax.fori_loop(0, S // RB, mlp_block, 0)
    for i in range(S // RB):
        out_copy(i).wait()


@jax.jit
def pallas_sequential_preLN__memory_aug_recurrent_mem_tr__mixer_s_mlp__prompt_kernel(
    A_x: jax.Array,
    A_mem0: jax.Array,
    A_Wq: jax.Array,
    A_Wk: jax.Array,
    A_Wv: jax.Array,
    A_Wo: jax.Array,
    A_seg_len: jax.Array,
    B_x: jax.Array,
    B_w1: jax.Array,
    B_w2: jax.Array,
    B_w3: jax.Array,
    B_w4: jax.Array,
):
    del A_seg_len, B_x
    hbm = pl.BlockSpec(memory_space=pl.ANY)
    vmem = pl.BlockSpec(memory_space=pltpu.VMEM)
    scratch = [
        pltpu.VMEM((H, D // 2, DH), u32),
        pltpu.VMEM((H, D // 2, DH), u32),
        pltpu.VMEM((H, D // 2, DH), u32),
        pltpu.VMEM((H * DH // 2, D), u32),
        pltpu.VMEM((D, 8, DH), bf16),
        pltpu.VMEM((D, 8, DH), bf16),
        pltpu.VMEM((D, 8, DH), bf16),
        pltpu.VMEM((S, D), bf16),
        pltpu.VMEM((S, D), f32),
        pltpu.VMEM((4, S + 2 * HALO, C4), f32),
        pltpu.VMEM((P0 // 2, D), u32),
        pltpu.VMEM((2 * TOK, D), u32),
        pltpu.VMEM((4, D, C4), bf16),
        pltpu.VMEM((D, D), bf16),
        pltpu.VMEM((D, F), bf16),
        pltpu.VMEM((F, D), bf16),
        pltpu.VMEM((S // 2, D), u32),
        pltpu.VMEM((RB // 2, FC), u32),
        pltpu.VMEM((RB // 2, FC), u32),
        pltpu.VMEM((RB, D), f32),
        pltpu.SemaphoreType.DMA((36,)),
    ] + [pltpu.VMEM((H // 8, RING, DH), f32)] * 24
    out = pl.pallas_call(
        _kernel,
        out_shape=jax.ShapeDtypeStruct((S, D), A_x.dtype),
        in_specs=[hbm, vmem] + [hbm] * 8,
        out_specs=hbm,
        scratch_shapes=scratch,
        compiler_params=pltpu.CompilerParams(vmem_limit_bytes=126 * 1024 * 1024),
    )(A_x.reshape(S, D), A_mem0.reshape(MEM, D), A_Wq, A_Wk, A_Wv,
      A_Wo.reshape(H * DH, D), B_w1, B_w2, B_w3, B_w4)
    return out.reshape(A_x.shape)
```

```python
import functools

import jax
import jax.numpy as jnp
from jax import lax
import jax.experimental.pallas as pl
import jax.experimental.pallas.tpu as pltpu

S = 2048
D = 1024
H = 32
DH = 128
MEM = 8
SEG = 32
F = 3584
NSEG = S // SEG
L = MEM + SEG
TOK = 24
P0 = S - TOK * NSEG
RING = 576
C4 = D // 4
HALO = 8
RB = 256
FC = 512
EPS = 1e-5
NEG = -1000000000.0

bf16 = jnp.bfloat16
f32 = jnp.float32
u32 = jnp.uint32

LAG_QK = 1
LAG_PV = 3
LAG_WO = 5
WO_GROUP = 1
import os as _os
_env = lambda k, d: int(_os.environ.get(k, d))
UNROLL = _env('UNROLL', 1)
LAG_QK = _env('LAG_QK', LAG_QK); LAG_PV = _env('LAG_PV', LAG_PV); LAG_WO = _env('LAG_WO', LAG_WO); WO_GROUP = _env('WO_GROUP', WO_GROUP)
SKIP_PRO = _env('SKIP_PRO', 0); SKIP_POST = _env('SKIP_POST', 0); SKIP_LOOP = _env('SKIP_LOOP', 0); SKIP_MLP = _env('SKIP_MLP', 0)
PAIRS = _env('PAIRS', 1)
PATTERN = _os.environ.get('PATTERN', 'asbfw')
NI = _env('NI', 8)
RELAY_SPAN = _env('RELAY_SPAN', 8)
START_AT = _env('START_AT', -1)
import contextlib
PROF = _env('PROF', 0)
class _Scopes:
    cur = None
    def __call__(self, name):
        if not PROF: return
        if self.cur is not None: self.cur.__exit__(None, None, None)
        self.cur = None
        if name is not None:
            self.cur = jax.named_scope(name); self.cur.__enter__()
F0_AT = _env('F0_AT', 17); F1_AT = _env('F1_AT', 18)


def _ln(x):
    m = jnp.mean(x, axis=-1, keepdims=True)
    d = x - m
    v = jnp.mean(d * d, axis=-1, keepdims=True)
    return d * lax.rsqrt(v + EPS)


def _gelu(x):
    return jax.nn.gelu(x, approximate=True)


def _pack(x):
    return pltpu.bitcast(x.astype(bf16), u32)


def _unpack(x):
    return pltpu.bitcast(x, bf16)


def _dot(a, b):
    return jnp.dot(a, b, preferred_element_type=f32)


def _kernel(x_hbm, mem0_ref, wq_hbm, wk_hbm, wv_hbm, wo_hbm, w1_hbm, w2_hbm,
            w3_hbm, w4_hbm, out_hbm,
            wq_s, wk_s, wv_s, wo_b, xs, hbuf, xg, ubuf,
            w1b, w2b, w3b, w4b, sems, *rings):
    scope = _Scopes()
    w_hbm = (wq_hbm, wk_hbm, wv_hbm)
    w_s = (wq_s, wk_s, wv_s)
    ring = [[rings[m * 8 + h % 8].at[h // 8] for h in range(H)] for m in range(3)]
    q_r, k_r, v_r = ring

    SEM_X0, SEM_X, SEM_WO, SEM_W1, SEM_W2, SEM_W3, SEM_W4, SEM_OUT, SEM_W = (
        0, 1, 13, 21, 25, 26, 27, 28, 36)
    XP = (S - P0) // 12

    x0_copy = pltpu.make_async_copy(x_hbm.at[pl.ds(0, P0)], xs.at[pl.ds(0, P0)],
                                    sems.at[SEM_X0])

    def x_copy(c):
        rows = pl.ds(pl.multiple_of(P0 + c * XP, XP), XP)
        return pltpu.make_async_copy(x_hbm.at[rows], xs.at[rows], sems.at[SEM_X + c])

    def wo_copy(i):
        rows = pl.ds(pl.multiple_of(i * 256, 256), 256)
        return pltpu.make_async_copy(wo_hbm.bitcast(u32).at[rows], wo_b.at[rows],
                                     sems.at[SEM_WO + i])

    def w1_copy(i):
        cols = pl.ds(pl.multiple_of(i * C4, C4), C4)
        return pltpu.make_async_copy(w1_hbm.bitcast(u32).at[:, cols], w1b.at[i],
                                     sems.at[SEM_W1 + i])

    w2_copy = pltpu.make_async_copy(w2_hbm.bitcast(u32), w2b, sems.at[SEM_W2])
    w3_copy = pltpu.make_async_copy(w3_hbm.bitcast(u32), w3b, sems.at[SEM_W3])
    w4_copy = pltpu.make_async_copy(w4_hbm.bitcast(u32), w4b, sems.at[SEM_W4])

    def mlp_weight_pieces(i):
        cps = []
        for src, dst, sem in ((w2_hbm, w2b, SEM_W2), (w3_hbm, w3b, SEM_W3),
                              (w4_hbm, w4b, SEM_W4)):
            n = dst.shape[0] // 8
            rows = pl.ds(pl.multiple_of(i * n, 8), n)
            cps.append(pltpu.make_async_copy(src.bitcast(u32).at[rows], dst.at[rows],
                                             sems.at[sem]))
        return cps

    def out_copy(i):
        rows = pl.ds(pl.multiple_of(i * RB, RB), RB)
        return pltpu.make_async_copy(xs.at[rows], out_hbm.at[rows], sems.at[SEM_OUT + i])

    def prologue(stg0, stg1, stg2, lhs0):
        stg = (stg0, stg1, stg2)

        def w_copies(g, m, kh):
            rows = pl.ds(pl.multiple_of(kh * (D // 4), D // 4), D // 4)
            src = w_hbm[m].bitcast(u32)
            dst = stg[m].reshape(D // 2, 8, DH)
            c = 3 * g + m
            return [pltpu.make_async_copy(
                src.at[rows, pl.ds(pl.multiple_of(16 * par + 4 * g, 4), 4), :],
                dst.at[rows, pl.ds(4 * par, 4), :],
                sems.at[SEM_W + 4 * c + 2 * kh + par]) for par in range(2)]

        def start(copies):
            for cp in copies:
                cp.start()

        def wait(copies):
            for cp in copies:
                cp.wait()

        def relayout(g, m, pair, i0, n):
            ev = stg[m][pl.ds(8 * i0 + pair, n, stride=8), :]
            od = stg[m][pl.ds(8 * i0 + 4 + pair, n, stride=8), :]
            h = 8 * g + 2 * pair
            w_s[m][h, pl.ds(i0, n), :] = (ev & jnp.uint32(0xFFFF)) | (od << 16)
            w_s[m][h + 1, pl.ds(i0, n), :] = (ev >> 16) | (od & jnp.uint32(0xFFFF0000))

        def norm_rows(r0, n, to_lhs0):
            xv = xs[pl.ds(r0, n), :].astype(f32)
            hbuf[pl.ds(r0, n), :] = xv
            xn = _ln(xv)
            if to_lhs0:
                lhs0[pl.ds(pl.multiple_of(r0 // 2, n // 2), n // 2), :] = _pack(xn)
            else:
                for c in range(4):
                    xg[c, pl.ds(HALO + r0, n), :] = xn[:, c * C4:(c + 1) * C4]

        scope('s00_init')
        x0_copy.start()
        start(w_copies(0, 0, 0))
        start(w_copies(0, 0, 1))
        x_copy(0).start()
        start(w_copies(0, 1, 0))
        start(w_copies(0, 1, 1))
        zero = jnp.zeros((HALO, C4), f32)
        for c in range(4):
            xg[c, pl.ds(0, HALO), :] = zero
            xg[c, pl.ds(HALO + S, HALO), :] = zero
        x0_copy.wait()
        scope('s01_norm0')

        @pl.loop(0, P0 // 128)
        def _(i):
            norm_rows(pl.multiple_of(i * 128, 128), 128, True)

        scope('s02_waitw0')
        wait(w_copies(0, 0, 0))
        wait(w_copies(0, 0, 1))
        scope('s03_rel0')

        @pl.loop(0, 4)
        def _(pair):
            for i0 in range(0, D // 2, 64):
                relayout(0, 0, pair, i0, 64)


        def stage(c, half, g, m):
            m1, m2 = (m + 1) % 3, (m + 2) % 3
            g1 = jnp.minimum(g + (1 if m == 2 else 0), 3)
            g2 = g + (1 if m >= 1 else 0)
            first = half == 0
            hp = P0 // 2
            r0 = pl.multiple_of(half * hp, hp)
            pieces = [(pair, i0) for i0 in range(0, D // 4, NI) for pair in range(4)]
            lo = 8 - RELAY_SPAN
            cuts = [len(pieces) * k // RELAY_SPAN for k in range(RELAY_SPAN + 1)]
            nr = XP // 8

            def dmas():
                @pl.when(first)
                def _():
                    x_copy(c).wait()

                @pl.when(c < 11)
                def _():
                    wait(w_copies(g1, m1, half))

            def dma_starts():
                @pl.when(first & (c < 10))
                def _():
                    start(w_copies(g2, m2, 0))
                    start(w_copies(g2, m2, 1))

                @pl.when(first & (c < 11))
                def _():
                    x_copy(c + 1).start()

                @pl.when(first & (c < 8))
                def _():
                    wo_copy(c).start()

                @pl.when(first & (c >= 8))
                def _():
                    w1_copy(c - 8).start()

            for j in range(8):
                if j == lo:
                    dmas()
                    if START_AT < 0:
                        dma_starts()
                if j >= lo:
                    for pair, i0 in pieces[cuts[j - lo]:cuts[j - lo + 1]]:
                        relayout(g1, m1, pair, pl.multiple_of(half * (D // 4) + i0, NI), NI)
                if j >= 4:
                    norm_rows(pl.multiple_of(
                        P0 + (2 * c + half) * (XP // 2) + (j - 4) * nr, nr), nr, False)
                lhs = _unpack(lhs0[pl.ds(pl.multiple_of(half * (hp // 2), hp // 2), hp // 2), :])
                res = _dot(lhs, _unpack(w_s[m][8 * g + j]))
                rings[m * 8 + j][g, pl.ds(r0, hp), :] = res
                if j == START_AT:
                    dma_starts()

        def stages(i, carry):
            c = i // 2
            half = i - 2 * c
            g = c // 3
            if PROF > 1: scope('s04b_stage')
            for m in range(3):
                pl.when(c - 3 * g == m)(functools.partial(stage, c, half, g, m))
            if PROF > 1: scope(None)
            return carry

        scope('s04_stages')
        lax.fori_loop(0, 24, stages, 0)
        scope(None)

    if not SKIP_PRO:
        pl.run_scoped(
            prologue,
            pltpu.VMEM((8 * D // 2, DH), u32),
            pltpu.VMEM((8 * D // 2, DH), u32),
            pltpu.VMEM((8 * D // 2, DH), u32),
            pltpu.VMEM((P0 // 2, D), u32),
        )
        scope('s05_waitwo')
        for i in range(8):
            wo_copy(i).wait()
        for i in range(4):
            w1_copy(i).wait()

    def wrap(r):
        return jnp.where(r >= RING, r - RING, r)

    def load_tok(s):
        t_tok = pl.multiple_of(HALO + P0 + TOK * s, 8)
        return jnp.concatenate([xg[c, pl.ds(t_tok, TOK), :] for c in range(4)], axis=1)

    def step(s, carry, tok):
        mem, rp, ra, rw = carry

        if not SKIP_PRO:
            @pl.when(s < 8)
            def _():
                for cp in mlp_weight_pieces(s):
                    cp.start()

        ri = lax.broadcasted_iota(jnp.int32, (L, L), 0)
        ci = lax.broadcasted_iota(jnp.int32, (L, L), 1)
        mask = (ri < MEM) | (ri >= ci)

        lhs = jnp.concatenate([mem, tok], axis=0).astype(bf16)
        rps = [pl.multiple_of(wrap(rp + 8 * i), 8) for i in range(3)]
        ra_ = pl.multiple_of(ra, SEG)
        rw_ = pl.multiple_of(rw, 8)

        col = s & 3
        rb = pl.multiple_of(jnp.maximum((s >> 2) - 1, 0) * (4 * TOK), 8)
        ubuf[...] = _pack(_ln(_ln(hbuf[pl.ds(rb, 4 * TOK), :])))

        def filler(j):
            u = _unpack(ubuf[...])
            r = _dot(u, _unpack(w1b[col, :, pl.ds(j * 128, 128)]))
            xg[col, pl.ds(HALO + rb, 4 * TOK), pl.ds(j * 128, 128)] = _gelu(r)

        mem_qkv = {}
        scores = {}
        o_mem = {}
        total = [None]

        def qkv(h):
            res = []
            for m in range(3):
                r = _dot(lhs, _unpack(w_s[m][h]))
                for i in range(3):
                    ring[m][h][pl.ds(rps[i], 8), :] = r[8 + 8 * i:16 + 8 * i]
                res.append(r[:MEM])
            mem_qkv[h] = res

        def qk(h):
            qm, km, vm = mem_qkv.pop(h)
            qa = jnp.concatenate([qm, q_r[h][pl.ds(ra_, SEG), :]], axis=0).astype(bf16)
            ka = jnp.concatenate([km, k_r[h][pl.ds(ra_, SEG), :]], axis=0).astype(bf16)
            sc = lax.dot_general(qa, ka, (((1,), (1,)), ((), ())),
                                 preferred_element_type=f32)
            scores[h] = (sc, vm)

        def pv(h):
            sc, vm = scores.pop(h)
            va = jnp.concatenate([vm, v_r[h][pl.ds(ra_, SEG), :]], axis=0).astype(bf16)
            sc = jnp.where(mask, sc * (DH ** -0.5), NEG)
            mx = jnp.max(sc, axis=1, keepdims=True)
            e = jnp.exp(sc - mx)
            den = jnp.sum(e, axis=1, keepdims=True)
            inv = pl.reciprocal(den, approx=True)
            inv = inv * (2.0 - den * inv)
            o = _dot(e.astype(bf16), va) * inv
            q_r[h][pl.ds(ra_, SEG), :] = o[MEM:]
            o_mem[h] = o[:MEM]

        def wo(g):
            hs = range(g * WO_GROUP, (g + 1) * WO_GROUP)
            lo = jnp.concatenate(
                [jnp.concatenate([o_mem.pop(h), q_r[h][pl.ds(rw_, TOK), :]], axis=0)
                 for h in hs], axis=1).astype(bf16)
            w = _unpack(wo_b[pl.ds(g * WO_GROUP * DH // 2, WO_GROUP * DH // 2), :])
            r = _dot(lo, w)
            total[0] = r if total[0] is None else total[0] + r

        if PAIRS:
            npair = H // 2
            t = 0
            nwo = 0
            while nwo < npair:
                for item in PATTERN:
                    if item == 'a' and t < npair:
                        qkv(2 * t)
                    if item == 'b' and t < npair:
                        qkv(2 * t + 1)
                    if item == 's':
                        if 0 <= t - LAG_QK < npair:
                            qk(2 * (t - LAG_QK))
                            qk(2 * (t - LAG_QK) + 1)
                        if 0 <= t - LAG_PV < npair:
                            pv(2 * (t - LAG_PV))
                            pv(2 * (t - LAG_PV) + 1)
                    if item == 'w' and 0 <= t - LAG_WO < npair:
                        wo(2 * (t - LAG_WO))
                        wo(2 * (t - LAG_WO) + 1)
                        nwo += 1
                    if item == 'f':
                        if t == F0_AT:
                            filler(0)
                        if t == F1_AT:
                            filler(1)
                t += 1
            if F1_AT < 0:
                filler(1)
        else:
            ng = H // WO_GROUP
            nxt = 0
            done_pv = 0
            t = 0
            while nxt < ng:
                if t < H:
                    qkv(t)
                if 0 <= t - LAG_QK < H:
                    qk(t - LAG_QK)
                if t == F0_AT:
                    filler(0)
                if t == F1_AT:
                    filler(1)
                if 0 <= t - LAG_PV < H:
                    pv(t - LAG_PV)
                    done_pv = t - LAG_PV + 1
                while (nxt < ng and t >= (nxt + 1) * WO_GROUP - 1 + LAG_WO
                       and done_pv >= (nxt + 1) * WO_GROUP):
                    wo(nxt)
                    nxt += 1
                t += 1
            if F1_AT < 0:
                filler(1)

        a = total[0]
        hr = pl.multiple_of(TOK * s, 8)
        hbuf[pl.ds(hr, TOK), :] += a[MEM:]
        return a[:MEM], wrap(rp + TOK), wrap(ra + SEG), wrap(rw + TOK)

    def steps(i, carry):
        if PROF > 1: scope('s06b_step')
        toks = [load_tok(i * UNROLL + k) for k in range(UNROLL)]
        for k in range(UNROLL):
            carry = step(i * UNROLL + k, carry, toks[k])
        if PROF > 1: scope(None)
        return carry

    scope('s06_loop')
    if not SKIP_LOOP: lax.fori_loop(
        0, NSEG // UNROLL, steps,
        (mem0_ref[...].astype(f32), jnp.int32(P0), jnp.int32(0), jnp.int32(0)))

    scope(None)
    def tail(yall, t0, t1, acc):
        scope('s07_post')
        if not SKIP_PRO:
            w2_copy.wait()
            w3_copy.wait()
            w4_copy.wait()
        if not SKIP_POST:

            def wo_batch(r0, n):
                rr = r0 % RING
                lo = jnp.concatenate(
                    [q_r[h][pl.ds(rr, n), :].astype(bf16) for h in range(H)], axis=1)
                hbuf[pl.ds(r0, n), :] += _dot(lo, _unpack(wo_b[...]))

            def mixer_in(r0, n):
                u = _ln(_ln(hbuf[pl.ds(r0, n), :])).astype(bf16)
                for c in range(4):
                    xg[c, pl.ds(HALO + r0, n), :] = _gelu(_dot(u, _unpack(w1b[c])))

            def mixer_out(i):
                r0 = i * RB
                parts = []
                for c, off in enumerate((-1, 1, -2, 2)):
                    win = xg[c, pl.ds(r0, RB + 2 * HALO), :]
                    parts.append(win[HALO + off:HALO + off + RB])
                hs = _dot(jnp.concatenate(parts, axis=1).astype(bf16), _unpack(w2b[...]))
                hv = hbuf[pl.ds(r0, RB), :]
                x1 = _ln(hv) + hs
                yall[pl.ds(r0 // 2, RB // 2), :] = _pack(_ln(x1))
                hbuf[pl.ds(r0, RB), :] = hv + x1

            done = TOK * NSEG
            split = 3 * RING
            first = 4 * TOK * (NSEG // 4 - 1)
            wo_batch(done, split - done)
            wo_batch(split, S - split)
            mixer_out(0)
            mixer_in(first, split - first)
            mixer_out(1)
            mixer_in(split, S - split)
            for i in range(2, S // RB):
                mixer_out(i)

        scope('s08_mlp')
        ts = (t0, t1)
        nc = F // FC

        def mlp_block(i, carry):
            rows = pl.ds(pl.multiple_of(i * RB, RB), RB)

            def up(c):
                y = _unpack(yall[pl.ds(pl.multiple_of(i * (RB // 2), RB // 2), RB // 2), :])
                r = _dot(y, _unpack(w3b[:, c * FC:(c + 1) * FC]))
                ts[c % 2][...] = _pack(_gelu(r))

            def down(c):
                r = _dot(_unpack(ts[c % 2][...]),
                         _unpack(w4b[c * FC // 2:(c + 1) * FC // 2, :]))
                if c == 0:
                    acc[...] = hbuf[rows, :] + r
                elif c < nc - 1:
                    acc[...] += r
                else:
                    xs[rows, :] = (acc[...] + r).astype(bf16)

            up(0)
            for c in range(nc):
                if c + 1 < nc:
                    up(c + 1)
                down(c)
            out_copy(i).start()
            return carry

        if not SKIP_MLP:
            lax.fori_loop(0, S // RB, mlp_block, 0)
            scope('s09_outwait')
            for i in range(S // RB):
                out_copy(i).wait()
        scope(None)

    pl.run_scoped(
        tail,
        pltpu.VMEM((S // 2, D), u32),
        pltpu.VMEM((RB // 2, FC), u32),
        pltpu.VMEM((RB // 2, FC), u32),
        pltpu.VMEM((RB, D), f32),
    )


@jax.jit
def pallas_sequential_preLN__memory_aug_recurrent_mem_tr__mixer_s_mlp__prompt_kernel(
    A_x: jax.Array,
    A_mem0: jax.Array,
    A_Wq: jax.Array,
    A_Wk: jax.Array,
    A_Wv: jax.Array,
    A_Wo: jax.Array,
    A_seg_len: jax.Array,
    B_x: jax.Array,
    B_w1: jax.Array,
    B_w2: jax.Array,
    B_w3: jax.Array,
    B_w4: jax.Array,
):
    del A_seg_len, B_x
    hbm = pl.BlockSpec(memory_space=pl.ANY)
    vmem = pl.BlockSpec(memory_space=pltpu.VMEM)
    scratch = [
        pltpu.VMEM((H, D // 2, DH), u32),
        pltpu.VMEM((H, D // 2, DH), u32),
        pltpu.VMEM((H, D // 2, DH), u32),
        pltpu.VMEM((H * DH // 2, D), u32),
        pltpu.VMEM((S, D), bf16),
        pltpu.VMEM((S, D), f32),
        pltpu.VMEM((4, S + 2 * HALO, C4), f32),
        pltpu.VMEM((2 * TOK, D), u32),
        pltpu.VMEM((4, D // 2, C4), u32),
        pltpu.VMEM((D // 2, D), u32),
        pltpu.VMEM((D // 2, F), u32),
        pltpu.VMEM((F // 2, D), u32),
        pltpu.SemaphoreType.DMA((84,)),
    ] + [pltpu.VMEM((H // 8, RING, DH), f32)] * 24
    out = pl.pallas_call(
        _kernel,
        out_shape=jax.ShapeDtypeStruct((S, D), A_x.dtype),
        in_specs=[hbm, vmem] + [hbm] * 8,
        out_specs=hbm,
        scratch_shapes=scratch,
        compiler_params=pltpu.CompilerParams(vmem_limit_bytes=126 * 1024 * 1024),
    )(A_x.reshape(S, D), A_mem0.reshape(MEM, D),
      A_Wq.reshape(D // 2, 2 * H, DH), A_Wk.reshape(D // 2, 2 * H, DH),
      A_Wv.reshape(D // 2, 2 * H, DH),
      A_Wo.reshape(H * DH, D), B_w1, B_w2, B_w3, B_w4)
    return out.reshape(A_x.shape)
```

```python
import functools

import jax
import jax.numpy as jnp
from jax import lax
import jax.experimental.pallas as pl
import jax.experimental.pallas.tpu as pltpu

S = 2048
D = 1024
H = 32
DH = 128
MEM = 8
SEG = 32
F = 3584
NSEG = S // SEG
L = MEM + SEG
TOK = 24
P0 = S - TOK * NSEG
RING = 576
C4 = D // 4
HALO = 8
RB = 256
FC = 512
EPS = 1e-5
NEG = -1000000000.0

bf16 = jnp.bfloat16
f32 = jnp.float32
u32 = jnp.uint32

LAG_QK = 1
LAG_PV = 3
LAG_WO = 5
WO_GROUP = 1
import os as _os
_env = lambda k, d: int(_os.environ.get(k, d))
UNROLL = _env('UNROLL', 2)
LAG_QK = _env('LAG_QK', LAG_QK); LAG_PV = _env('LAG_PV', LAG_PV); LAG_WO = _env('LAG_WO', LAG_WO); WO_GROUP = _env('WO_GROUP', WO_GROUP)
SKIP_PRO = _env('SKIP_PRO', 0); SKIP_POST = _env('SKIP_POST', 0); SKIP_LOOP = _env('SKIP_LOOP', 0); SKIP_MLP = _env('SKIP_MLP', 0)
PAIRS = _env('PAIRS', 1)
PATTERN = _os.environ.get('PATTERN', 'asbfw')
NI = _env('NI', 8)
RELAY_SPAN = _env('RELAY_SPAN', 8)
WAIT_AT = _env('WAIT_AT', 5)
import contextlib
PROF = _env('PROF', 0)
class _Scopes:
    cur = None
    def __call__(self, name):
        if not PROF: return
        if self.cur is not None: self.cur.__exit__(None, None, None)
        self.cur = None
        if name is not None:
            self.cur = jax.named_scope(name); self.cur.__enter__()
F0_AT = _env('F0_AT', 17); F1_AT = _env('F1_AT', -1)


def mult(i, n):
    return i if isinstance(i, int) else pl.multiple_of(i, n)


def _ln(x):
    m = jnp.mean(x, axis=-1, keepdims=True)
    d = x - m
    v = jnp.mean(d * d, axis=-1, keepdims=True)
    return d * lax.rsqrt(v + EPS)


def _gelu(x):
    return jax.nn.gelu(x, approximate=True)


def _pack(x):
    return pltpu.bitcast(x.astype(bf16), u32)


def _unpack(x):
    return pltpu.bitcast(x, bf16)


def _dot(a, b):
    return jnp.dot(a, b, preferred_element_type=f32)


def _kernel(x_hbm, mem0_ref, wq_hbm, wk_hbm, wv_hbm, wo_hbm, w1_hbm, w2_hbm,
            w3_hbm, w4_hbm, out_hbm,
            wq_s, wk_s, wv_s, wo_b, xs, hbuf, xg, ubuf,
            w1b, w2b, w3b, w4b, sems, *rings):
    scope = _Scopes()
    w_hbm = (wq_hbm, wk_hbm, wv_hbm)
    w_s = (wq_s, wk_s, wv_s)
    ring = [[rings[m * 8 + h % 8].at[h // 8] for h in range(H)] for m in range(3)]
    q_r, k_r, v_r = ring

    SEM_X0, SEM_X, SEM_WO, SEM_W1, SEM_W2, SEM_W3, SEM_W4, SEM_OUT, SEM_W = (
        0, 1, 13, 21, 25, 26, 27, 28, 36)
    XP = (S - P0) // 12

    x0_copy = pltpu.make_async_copy(x_hbm.at[pl.ds(0, P0)], xs.at[pl.ds(0, P0)],
                                    sems.at[SEM_X0])

    def x_copy(g):
        rows = pl.ds(mult(P0 + g * 3 * XP, XP), 3 * XP)
        return pltpu.make_async_copy(x_hbm.at[rows], xs.at[rows], sems.at[SEM_X + g])

    def wo_copy(i):
        rows = pl.ds(mult(i * 512, 512), 512)
        return pltpu.make_async_copy(wo_hbm.bitcast(u32).at[rows], wo_b.at[rows],
                                     sems.at[SEM_WO + i])

    def w1_copy(i):
        cols = pl.ds(mult(i * C4, C4), C4)
        return pltpu.make_async_copy(w1_hbm.bitcast(u32).at[:, cols], w1b.at[i],
                                     sems.at[SEM_W1 + i])

    w2_copy = pltpu.make_async_copy(w2_hbm.bitcast(u32), w2b, sems.at[SEM_W2])
    w3_copy = pltpu.make_async_copy(w3_hbm.bitcast(u32), w3b, sems.at[SEM_W3])
    w4_copy = pltpu.make_async_copy(w4_hbm.bitcast(u32), w4b, sems.at[SEM_W4])

    def out_copy(i):
        rows = pl.ds(pl.multiple_of(i * RB, RB), RB)
        return pltpu.make_async_copy(xs.at[rows], out_hbm.at[rows], sems.at[SEM_OUT + i])

    def prologue(stg0, stg1, stg2, lhs0):
        stg = (stg0, stg1, stg2)

        def w_copies(g, m):
            src = w_hbm[m].bitcast(u32)
            dst = stg[m].reshape(D // 2, 8, DH)
            return [pltpu.make_async_copy(
                src.at[:, pl.ds(pl.multiple_of(16 * par + 4 * g, 4), 4), :],
                dst.at[:, pl.ds(4 * par, 4), :],
                sems.at[SEM_W + 3 * g + m]) for par in range(2)]

        def start(copies):
            for cp in copies:
                cp.start()

        def wait(copies):
            for cp in copies:
                cp.wait()

        def relayout(g, m, pair, i0, n):
            ev = stg[m][pl.ds(8 * i0 + pair, n, stride=8), :]
            od = stg[m][pl.ds(8 * i0 + 4 + pair, n, stride=8), :]
            h = 8 * g + 2 * pair
            w_s[m][h, pl.ds(i0, n), :] = (ev & jnp.uint32(0xFFFF)) | (od << 16)
            w_s[m][h + 1, pl.ds(i0, n), :] = (ev >> 16) | (od & jnp.uint32(0xFFFF0000))

        def norm_rows(r0, n, to_lhs0):
            xv = xs[pl.ds(r0, n), :].astype(f32)
            hbuf[pl.ds(r0, n), :] = xv
            xn = _ln(xv)
            if to_lhs0:
                lhs0[pl.ds(pl.multiple_of(r0 // 2, n // 2), n // 2), :] = _pack(xn)
            else:
                for c in range(4):
                    xg[c, pl.ds(HALO + r0, n), :] = xn[:, c * C4:(c + 1) * C4]

        scope('s00_init')
        x0_copy.start()
        start(w_copies(0, 0))
        start(w_copies(0, 1))
        x_copy(0).start()
        start(w_copies(0, 2))
        w1_copy(0).start()
        zero = jnp.zeros((HALO, C4), f32)
        for c in range(4):
            xg[c, pl.ds(0, HALO), :] = zero
            xg[c, pl.ds(HALO + S, HALO), :] = zero
        x0_copy.wait()
        scope('s01_norm0')

        @pl.loop(0, P0 // 128)
        def _(i):
            norm_rows(pl.multiple_of(i * 128, 128), 128, True)

        scope('s02_waitw0')
        pltpu.make_async_copy(stg[0], stg[0], sems.at[SEM_W]).wait()
        scope('s03_rel0')

        @pl.loop(0, 4)
        def _(pair):
            for i0 in range(0, D // 2, 64):
                relayout(0, 0, pair, i0, 64)


        def stage(c, g, m):
            m1 = (m + 1) % 3
            g1 = jnp.minimum(g + (1 if m == 2 else 0), 3)
            pieces = [(pair, i0) for i0 in range(0, D // 2, NI) for pair in range(4)]
            span = 8 - WAIT_AT
            cuts = [len(pieces) * k // span for k in range(span + 1)]
            rcuts = [XP // 16 * k // span * 16 for k in range(span + 1)]

            def waits():
                @pl.when(c < 11)
                def _():
                    pltpu.make_async_copy(stg[m1], stg[m1],
                                          sems.at[SEM_W + 3 * g1 + m1]).wait()
                if m == 0:
                    x_copy(g).wait()

            def starts():
                @pl.when(g < 3)
                def _():
                    start(w_copies(g + 1, m))
                    if m == 0:
                        x_copy(g + 1).start()
                    if m == 2:
                        w1_copy(g + 1).start()
                if m == 1:
                    wo_copy(g).start()

            for j in range(8):
                if j >= WAIT_AT:
                    k = j - WAIT_AT
                    for pair, i0 in pieces[cuts[k]:cuts[k + 1]]:
                        relayout(g1, m1, pair, i0, NI)
                    nr = rcuts[k + 1] - rcuts[k]
                    if nr:
                        norm_rows(pl.multiple_of(P0 + c * XP + rcuts[k], 16), nr, False)
                res = _dot(_unpack(lhs0[...]), _unpack(w_s[m][8 * g + j]))
                if j == WAIT_AT - 1:
                    waits()
                if j == 7:
                    starts()
                rings[m * 8 + j][g, pl.ds(0, P0), :] = res

        def stages(c, carry):
            g = c // 3
            if PROF > 1: scope('s04b_stage')
            for m in range(3):
                pl.when(c - 3 * g == m)(functools.partial(stage, c, g, m))
            if PROF > 1: scope(None)
            return carry

        scope('s04_stages')
        lax.fori_loop(0, 12, stages, 0)
        scope(None)

    if not SKIP_PRO:
        pl.run_scoped(
            prologue,
            pltpu.VMEM((8 * D // 2, DH), u32),
            pltpu.VMEM((8 * D // 2, DH), u32),
            pltpu.VMEM((8 * D // 2, DH), u32),
            pltpu.VMEM((P0 // 2, D), u32),
        )
        scope('s05_waitwo')
        w2_copy.start()
        w3_copy.start()
        w4_copy.start()
        for i in range(4):
            wo_copy(i).wait()
        for i in range(4):
            w1_copy(i).wait()

    def wrap(r):
        return jnp.where(r >= RING, r - RING, r)

    def load_tok(s):
        t_tok = pl.multiple_of(HALO + P0 + TOK * s, 8)
        return jnp.concatenate([xg[c, pl.ds(t_tok, TOK), :] for c in range(4)], axis=1)

    def step(s, carry, tok):
        mem, rp, ra, rw = carry

        ri = lax.broadcasted_iota(jnp.int32, (L, L), 0)
        ci = lax.broadcasted_iota(jnp.int32, (L, L), 1)
        mask = (ri < MEM) | (ri >= ci)

        lhs = jnp.concatenate([mem, tok], axis=0).astype(bf16)
        rps = [pl.multiple_of(wrap(rp + 8 * i), 8) for i in range(3)]
        ra_ = pl.multiple_of(ra, SEG)
        rw_ = pl.multiple_of(rw, 8)

        col = s & 3
        rb = pl.multiple_of(jnp.maximum((s >> 2) - 1, 0) * (4 * TOK), 8)
        ubuf[...] = _pack(_ln(_ln(hbuf[pl.ds(rb, 4 * TOK), :])))

        def filler(j):
            u = _unpack(ubuf[...])
            r = _dot(u, _unpack(w1b[col, :, pl.ds(j * 128, 128)]))
            xg[col, pl.ds(HALO + rb, 4 * TOK), pl.ds(j * 128, 128)] = _gelu(r)

        mem_qkv = {}
        scores = {}
        o_mem = {}
        total = [None]

        def qkv(h):
            res = []
            for m in range(3):
                r = _dot(lhs, _unpack(w_s[m][h]))
                for i in range(3):
                    ring[m][h][pl.ds(rps[i], 8), :] = r[8 + 8 * i:16 + 8 * i]
                res.append(r[:MEM])
            mem_qkv[h] = res

        def qk(h):
            qm, km, vm = mem_qkv.pop(h)
            qa = jnp.concatenate([qm, q_r[h][pl.ds(ra_, SEG), :]], axis=0).astype(bf16)
            ka = jnp.concatenate([km, k_r[h][pl.ds(ra_, SEG), :]], axis=0).astype(bf16)
            sc = lax.dot_general(qa, ka, (((1,), (1,)), ((), ())),
                                 preferred_element_type=f32)
            scores[h] = (sc, vm)

        def pv(h):
            sc, vm = scores.pop(h)
            va = jnp.concatenate([vm, v_r[h][pl.ds(ra_, SEG), :]], axis=0).astype(bf16)
            sc = jnp.where(mask, sc * (DH ** -0.5), NEG)
            mx = jnp.max(sc, axis=1, keepdims=True)
            e = jnp.exp(sc - mx)
            den = jnp.sum(e, axis=1, keepdims=True)
            inv = pl.reciprocal(den, approx=True)
            inv = inv * (2.0 - den * inv)
            o = _dot(e.astype(bf16), va) * inv
            q_r[h][pl.ds(ra_, SEG), :] = o[MEM:]
            o_mem[h] = o[:MEM]

        def wo(g):
            hs = range(g * WO_GROUP, (g + 1) * WO_GROUP)
            lo = jnp.concatenate(
                [jnp.concatenate([o_mem.pop(h), q_r[h][pl.ds(rw_, TOK), :]], axis=0)
                 for h in hs], axis=1).astype(bf16)
            w = _unpack(wo_b[pl.ds(g * WO_GROUP * DH // 2, WO_GROUP * DH // 2), :])
            r = _dot(lo, w)
            total[0] = r if total[0] is None else total[0] + r

        if PAIRS:
            npair = H // 2
            t = 0
            nwo = 0
            while nwo < npair:
                for item in PATTERN:
                    if item == 'a' and t < npair:
                        qkv(2 * t)
                    if item == 'b' and t < npair:
                        qkv(2 * t + 1)
                    if item == 's':
                        if 0 <= t - LAG_QK < npair:
                            qk(2 * (t - LAG_QK))
                            qk(2 * (t - LAG_QK) + 1)
                        if 0 <= t - LAG_PV < npair:
                            pv(2 * (t - LAG_PV))
                            pv(2 * (t - LAG_PV) + 1)
                    if item == 'w' and 0 <= t - LAG_WO < npair:
                        wo(2 * (t - LAG_WO))
                        wo(2 * (t - LAG_WO) + 1)
                        nwo += 1
                    if item == 'f':
                        if t == F0_AT:
                            filler(0)
                        if t == F1_AT:
                            filler(1)
                t += 1
            if F1_AT < 0:
                filler(1)
        else:
            ng = H // WO_GROUP
            nxt = 0
            done_pv = 0
            t = 0
            while nxt < ng:
                if t < H:
                    qkv(t)
                if 0 <= t - LAG_QK < H:
                    qk(t - LAG_QK)
                if t == F0_AT:
                    filler(0)
                if t == F1_AT:
                    filler(1)
                if 0 <= t - LAG_PV < H:
                    pv(t - LAG_PV)
                    done_pv = t - LAG_PV + 1
                while (nxt < ng and t >= (nxt + 1) * WO_GROUP - 1 + LAG_WO
                       and done_pv >= (nxt + 1) * WO_GROUP):
                    wo(nxt)
                    nxt += 1
                t += 1
            if F1_AT < 0:
                filler(1)

        a = total[0]
        hr = pl.multiple_of(TOK * s, 8)
        hbuf[pl.ds(hr, TOK), :] += a[MEM:]
        return a[:MEM], wrap(rp + TOK), wrap(ra + SEG), wrap(rw + TOK)

    def steps(i, carry):
        if PROF > 1: scope('s06b_step')
        toks = [load_tok(i * UNROLL + k) for k in range(UNROLL)]
        for k in range(UNROLL):
            carry = step(i * UNROLL + k, carry, toks[k])
        if PROF > 1: scope(None)
        return carry

    scope('s06_loop')
    if not SKIP_LOOP: lax.fori_loop(
        0, NSEG // UNROLL, steps,
        (mem0_ref[...].astype(f32), jnp.int32(P0), jnp.int32(0), jnp.int32(0)))

    scope(None)
    def tail(yall, t0, t1, acc):
        scope('s07_post')
        if not SKIP_PRO:
            w2_copy.wait()
            w3_copy.wait()
            w4_copy.wait()
        if not SKIP_POST:

            def wo_batch(r0, n):
                rr = r0 % RING
                lo = jnp.concatenate(
                    [q_r[h][pl.ds(rr, n), :].astype(bf16) for h in range(H)], axis=1)
                hbuf[pl.ds(r0, n), :] += _dot(lo, _unpack(wo_b[...]))

            def mixer_in(r0, n):
                u = _ln(_ln(hbuf[pl.ds(r0, n), :])).astype(bf16)
                for c in range(4):
                    xg[c, pl.ds(HALO + r0, n), :] = _gelu(_dot(u, _unpack(w1b[c])))

            def mixer_out(i):
                r0 = i * RB
                parts = []
                for c, off in enumerate((-1, 1, -2, 2)):
                    win = xg[c, pl.ds(r0, RB + 2 * HALO), :]
                    parts.append(win[HALO + off:HALO + off + RB])
                hs = _dot(jnp.concatenate(parts, axis=1).astype(bf16), _unpack(w2b[...]))
                hv = hbuf[pl.ds(r0, RB), :]
                x1 = _ln(hv) + hs
                yall[pl.ds(r0 // 2, RB // 2), :] = _pack(_ln(x1))
                hbuf[pl.ds(r0, RB), :] = hv + x1

            done = TOK * NSEG
            split = 3 * RING
            first = 4 * TOK * (NSEG // 4 - 1)
            wo_batch(done, split - done)
            wo_batch(split, S - split)
            mixer_out(0)
            mixer_in(first, split - first)
            mixer_out(1)
            mixer_in(split, S - split)
            for i in range(2, S // RB):
                mixer_out(i)

        scope('s08_mlp')
        ts = (t0, t1)
        nc = F // FC

        def mlp_block(i, carry):
            rows = pl.ds(pl.multiple_of(i * RB, RB), RB)

            def up(c):
                y = _unpack(yall[pl.ds(pl.multiple_of(i * (RB // 2), RB // 2), RB // 2), :])
                r = _dot(y, _unpack(w3b[:, c * FC:(c + 1) * FC]))
                ts[c % 2][...] = _pack(_gelu(r))

            def down(c):
                r = _dot(_unpack(ts[c % 2][...]),
                         _unpack(w4b[c * FC // 2:(c + 1) * FC // 2, :]))
                if c == 0:
                    acc[...] = hbuf[rows, :] + r
                elif c < nc - 1:
                    acc[...] += r
                else:
                    xs[rows, :] = (acc[...] + r).astype(bf16)

            up(0)
            for c in range(nc):
                if c + 1 < nc:
                    up(c + 1)
                down(c)
            out_copy(i).start()
            return carry

        if not SKIP_MLP:
            lax.fori_loop(0, S // RB, mlp_block, 0)
            scope('s09_outwait')
            for i in range(S // RB):
                out_copy(i).wait()
        scope(None)

    pl.run_scoped(
        tail,
        pltpu.VMEM((S // 2, D), u32),
        pltpu.VMEM((RB // 2, FC), u32),
        pltpu.VMEM((RB // 2, FC), u32),
        pltpu.VMEM((RB, D), f32),
    )


@jax.jit
def pallas_sequential_preLN__memory_aug_recurrent_mem_tr__mixer_s_mlp__prompt_kernel(
    A_x: jax.Array,
    A_mem0: jax.Array,
    A_Wq: jax.Array,
    A_Wk: jax.Array,
    A_Wv: jax.Array,
    A_Wo: jax.Array,
    A_seg_len: jax.Array,
    B_x: jax.Array,
    B_w1: jax.Array,
    B_w2: jax.Array,
    B_w3: jax.Array,
    B_w4: jax.Array,
):
    del A_seg_len, B_x
    hbm = pl.BlockSpec(memory_space=pl.ANY)
    vmem = pl.BlockSpec(memory_space=pltpu.VMEM)
    scratch = [
        pltpu.VMEM((H, D // 2, DH), u32),
        pltpu.VMEM((H, D // 2, DH), u32),
        pltpu.VMEM((H, D // 2, DH), u32),
        pltpu.VMEM((H * DH // 2, D), u32),
        pltpu.VMEM((S, D), bf16),
        pltpu.VMEM((S, D), f32),
        pltpu.VMEM((4, S + 2 * HALO, C4), f32),
        pltpu.VMEM((2 * TOK, D), u32),
        pltpu.VMEM((4, D // 2, C4), u32),
        pltpu.VMEM((D // 2, D), u32),
        pltpu.VMEM((D // 2, F), u32),
        pltpu.VMEM((F // 2, D), u32),
        pltpu.SemaphoreType.DMA((48,)),
    ] + [pltpu.VMEM((H // 8, RING, DH), f32)] * 24
    out = pl.pallas_call(
        _kernel,
        out_shape=jax.ShapeDtypeStruct((S, D), A_x.dtype),
        in_specs=[hbm, vmem] + [hbm] * 8,
        out_specs=hbm,
        scratch_shapes=scratch,
        compiler_params=pltpu.CompilerParams(vmem_limit_bytes=126 * 1024 * 1024),
    )(A_x.reshape(S, D), A_mem0.reshape(MEM, D),
      A_Wq.reshape(D // 2, 2 * H, DH), A_Wk.reshape(D // 2, 2 * H, DH),
      A_Wv.reshape(D // 2, 2 * H, DH),
      A_Wo.reshape(H * DH, D), B_w1, B_w2, B_w3, B_w4)
    return out.reshape(A_x.shape)
```

```python
import functools

import jax
import jax.numpy as jnp
from jax import lax
import jax.experimental.pallas as pl
import jax.experimental.pallas.tpu as pltpu

S = 2048
D = 1024
H = 32
DH = 128
MEM = 8
SEG = 32
F = 3584
NSEG = S // SEG
L = MEM + SEG
TOK = 24
P0 = S - TOK * NSEG
RING = 576
C4 = D // 4
HALO = 8
RB = 256
FC = 512
EPS = 1e-5
NEG = -1000000000.0

bf16 = jnp.bfloat16
f32 = jnp.float32
u32 = jnp.uint32

LAG_QK = 1
LAG_PV = 3
LAG_WO = 5
WO_GROUP = 1
import os as _os
_env = lambda k, d: int(_os.environ.get(k, d))
UNROLL = _env('UNROLL', 2)
LAG_QK = _env('LAG_QK', LAG_QK); LAG_PV = _env('LAG_PV', LAG_PV); LAG_WO = _env('LAG_WO', LAG_WO); WO_GROUP = _env('WO_GROUP', WO_GROUP)
SKIP_PRO = _env('SKIP_PRO', 0); SKIP_POST = _env('SKIP_POST', 0); SKIP_LOOP = _env('SKIP_LOOP', 0); SKIP_MLP = _env('SKIP_MLP', 0)
PAIRS = _env('PAIRS', 1)
PATTERN = _os.environ.get('PATTERN', 'asbfw')
KCH = _env('KCH', 1)
POSTORD = _os.environ.get('POSTORD', 'tATuBU01v2aVb3c45d6e7fgh')
NI = _env('NI', 8)
RELAY_SPAN = _env('RELAY_SPAN', 8)
WAIT_AT = _env('WAIT_AT', 5)
import contextlib
PROF = _env('PROF', 0)
class _Scopes:
    cur = None
    def __call__(self, name):
        if not PROF: return
        if self.cur is not None: self.cur.__exit__(None, None, None)
        self.cur = None
        if name is not None:
            self.cur = jax.named_scope(name); self.cur.__enter__()
F0_AT = _env('F0_AT', 17); F1_AT = _env('F1_AT', -1)


def mult(i, n):
    return i if isinstance(i, int) else pl.multiple_of(i, n)


def _ln(x):
    m = jnp.mean(x, axis=-1, keepdims=True)
    d = x - m
    v = jnp.mean(d * d, axis=-1, keepdims=True)
    return d * lax.rsqrt(v + EPS)


def _gelu(x):
    return jax.nn.gelu(x, approximate=True)


def _pack(x):
    return pltpu.bitcast(x.astype(bf16), u32)


def _unpack(x):
    return pltpu.bitcast(x, bf16)


def _dot(a, b):
    return jnp.dot(a, b, preferred_element_type=f32)


def _kernel(x_hbm, mem0_ref, wq_hbm, wk_hbm, wv_hbm, wo_hbm, w1_hbm, w2_hbm,
            w3_hbm, w4_hbm, out_hbm,
            wq_s, wk_s, wv_s, wo_b, xs, hbuf, xg, ubuf,
            w1b, w2b, w3b, w4b, sems, *rings):
    scope = _Scopes()
    w_hbm = (wq_hbm, wk_hbm, wv_hbm)
    w_s = (wq_s, wk_s, wv_s)
    ring = [[rings[m * 8 + h % 8].at[h // 8] for h in range(H)] for m in range(3)]
    q_r, k_r, v_r = ring

    SEM_X0, SEM_X, SEM_WO, SEM_W1, SEM_W2, SEM_W3, SEM_W4, SEM_OUT, SEM_W = (
        0, 1, 13, 21, 25, 26, 27, 28, 36)
    XP = (S - P0) // 12

    x0_copy = pltpu.make_async_copy(x_hbm.at[pl.ds(0, P0)], xs.at[pl.ds(0, P0)],
                                    sems.at[SEM_X0])

    def x_copy(g):
        rows = pl.ds(mult(P0 + g * 3 * XP, XP), 3 * XP)
        return pltpu.make_async_copy(x_hbm.at[rows], xs.at[rows], sems.at[SEM_X + g])

    def wo_copy(i):
        rows = pl.ds(mult(i * 512, 512), 512)
        return pltpu.make_async_copy(wo_hbm.bitcast(u32).at[rows], wo_b.at[rows],
                                     sems.at[SEM_WO + i])

    def w1_copy(i):
        cols = pl.ds(mult(i * C4, C4), C4)
        return pltpu.make_async_copy(w1_hbm.bitcast(u32).at[:, cols], w1b.at[i],
                                     sems.at[SEM_W1 + i])

    w2_copy = pltpu.make_async_copy(w2_hbm.bitcast(u32), w2b, sems.at[SEM_W2])
    w3_copy = pltpu.make_async_copy(w3_hbm.bitcast(u32), w3b, sems.at[SEM_W3])
    w4_copy = pltpu.make_async_copy(w4_hbm.bitcast(u32), w4b, sems.at[SEM_W4])

    def out_copy(i):
        rows = pl.ds(pl.multiple_of(i * RB, RB), RB)
        return pltpu.make_async_copy(xs.at[rows], out_hbm.at[rows], sems.at[SEM_OUT + i])

    def prologue(stg0, stg1, stg2, lhs0):
        stg = (stg0, stg1, stg2)

        def w_copies(g, m):
            src = w_hbm[m].bitcast(u32)
            dst = stg[m].reshape(D // 2, 8, DH)
            return [pltpu.make_async_copy(
                src.at[:, pl.ds(pl.multiple_of(16 * par + 4 * g, 4), 4), :],
                dst.at[:, pl.ds(4 * par, 4), :],
                sems.at[SEM_W + 3 * g + m]) for par in range(2)]

        def start(copies):
            for cp in copies:
                cp.start()

        def wait(copies):
            for cp in copies:
                cp.wait()

        def relayout(g, m, pair, i0, n):
            ev = stg[m][pl.ds(8 * i0 + pair, n, stride=8), :]
            od = stg[m][pl.ds(8 * i0 + 4 + pair, n, stride=8), :]
            h = 8 * g + 2 * pair
            w_s[m][h, pl.ds(i0, n), :] = (ev & jnp.uint32(0xFFFF)) | (od << 16)
            w_s[m][h + 1, pl.ds(i0, n), :] = (ev >> 16) | (od & jnp.uint32(0xFFFF0000))

        def norm_rows(r0, n, to_lhs0):
            xv = xs[pl.ds(r0, n), :].astype(f32)
            hbuf[pl.ds(r0, n), :] = xv
            xn = _ln(xv)
            if to_lhs0:
                lhs0[pl.ds(pl.multiple_of(r0 // 2, n // 2), n // 2), :] = _pack(xn)
            else:
                for c in range(4):
                    xg[c, pl.ds(HALO + r0, n), :] = xn[:, c * C4:(c + 1) * C4]

        scope('s00_init')
        x0_copy.start()
        start(w_copies(0, 0))
        start(w_copies(0, 1))
        x_copy(0).start()
        start(w_copies(0, 2))
        w1_copy(0).start()
        zero = jnp.zeros((HALO, C4), f32)
        for c in range(4):
            xg[c, pl.ds(0, HALO), :] = zero
            xg[c, pl.ds(HALO + S, HALO), :] = zero
        x0_copy.wait()
        scope('s01_norm0')

        @pl.loop(0, P0 // 128)
        def _(i):
            norm_rows(pl.multiple_of(i * 128, 128), 128, True)

        scope('s02_waitw0')
        pltpu.make_async_copy(stg[0], stg[0], sems.at[SEM_W]).wait()
        scope('s03_rel0')

        @pl.loop(0, 4)
        def _(pair):
            for i0 in range(0, D // 2, 64):
                relayout(0, 0, pair, i0, 64)


        def stage(c, g, m):
            m1 = (m + 1) % 3
            g1 = jnp.minimum(g + (1 if m == 2 else 0), 3)
            pieces = [(pair, i0) for i0 in range(0, D // 2, NI) for pair in range(4)]
            span = 8 - WAIT_AT
            cuts = [len(pieces) * k // span for k in range(span + 1)]
            rcuts = [XP // 16 * k // span * 16 for k in range(span + 1)]

            def waits():
                @pl.when(c < 11)
                def _():
                    pltpu.make_async_copy(stg[m1], stg[m1],
                                          sems.at[SEM_W + 3 * g1 + m1]).wait()
                if m == 0:
                    x_copy(g).wait()

            def starts():
                @pl.when(g < 3)
                def _():
                    start(w_copies(g + 1, m))
                    if m == 0:
                        x_copy(g + 1).start()
                    if m == 2:
                        w1_copy(g + 1).start()
                if m == 1:
                    wo_copy(g).start()

            for j in range(8):
                if j >= WAIT_AT:
                    k = j - WAIT_AT
                    for pair, i0 in pieces[cuts[k]:cuts[k + 1]]:
                        relayout(g1, m1, pair, i0, NI)
                    nr = rcuts[k + 1] - rcuts[k]
                    if nr:
                        norm_rows(pl.multiple_of(P0 + c * XP + rcuts[k], 16), nr, False)
                res = _dot(_unpack(lhs0[...]), _unpack(w_s[m][8 * g + j]))
                if j == WAIT_AT - 1:
                    waits()
                if j == 7:
                    starts()
                rings[m * 8 + j][g, pl.ds(0, P0), :] = res

        def stages(c, carry):
            g = c // 3
            if PROF > 1: scope('s04b_stage')
            for m in range(3):
                pl.when(c - 3 * g == m)(functools.partial(stage, c, g, m))
            if PROF > 1: scope(None)
            return carry

        scope('s04_stages')
        lax.fori_loop(0, 12, stages, 0)
        scope(None)

    if not SKIP_PRO:
        pl.run_scoped(
            prologue,
            pltpu.VMEM((8 * D // 2, DH), u32),
            pltpu.VMEM((8 * D // 2, DH), u32),
            pltpu.VMEM((8 * D // 2, DH), u32),
            pltpu.VMEM((P0 // 2, D), u32),
        )
        scope('s05_waitwo')
        w2_copy.start()
        w3_copy.start()
        w4_copy.start()
        for i in range(4):
            wo_copy(i).wait()
        for i in range(4):
            w1_copy(i).wait()

    def wrap(r):
        return jnp.where(r >= RING, r - RING, r)

    def load_tok(s):
        t_tok = pl.multiple_of(HALO + P0 + TOK * s, 8)
        return jnp.concatenate([xg[c, pl.ds(t_tok, TOK), :] for c in range(4)], axis=1)

    def step(s, carry, tok):
        mem, rp, ra, rw = carry

        ri = lax.broadcasted_iota(jnp.int32, (L, L), 0)
        ci = lax.broadcasted_iota(jnp.int32, (L, L), 1)
        mask = (ri < MEM) | (ri >= ci)

        lhs = jnp.concatenate([mem, tok], axis=0).astype(bf16)
        rps = [pl.multiple_of(wrap(rp + 8 * i), 8) for i in range(3)]
        ra_ = pl.multiple_of(ra, SEG)
        rw_ = pl.multiple_of(rw, 8)

        col = s & 3
        rb = pl.multiple_of(jnp.maximum((s >> 2) - 1, 0) * (4 * TOK), 8)
        ubuf[...] = _pack(_ln(_ln(hbuf[pl.ds(rb, 4 * TOK), :])))

        def filler(j):
            u = _unpack(ubuf[...])
            r = _dot(u, _unpack(w1b[col, :, pl.ds(j * 128, 128)]))
            xg[col, pl.ds(HALO + rb, 4 * TOK), pl.ds(j * 128, 128)] = _gelu(r)

        mem_qkv = {}
        scores = {}
        o_mem = {}
        total = [None]

        def qkv(h):
            res = []
            for m in range(3):
                r = _dot(lhs, _unpack(w_s[m][h]))
                for i in range(3):
                    ring[m][h][pl.ds(rps[i], 8), :] = r[8 + 8 * i:16 + 8 * i]
                res.append(r[:MEM])
            mem_qkv[h] = res

        def qk(h):
            qm, km, vm = mem_qkv.pop(h)
            qa = jnp.concatenate([qm, q_r[h][pl.ds(ra_, SEG), :]], axis=0).astype(bf16)
            ka = jnp.concatenate([km, k_r[h][pl.ds(ra_, SEG), :]], axis=0).astype(bf16)
            sc = lax.dot_general(qa, ka, (((1,), (1,)), ((), ())),
                                 preferred_element_type=f32)
            scores[h] = (sc, vm)

        def pv(h):
            sc, vm = scores.pop(h)
            va = jnp.concatenate([vm, v_r[h][pl.ds(ra_, SEG), :]], axis=0).astype(bf16)
            sc = jnp.where(mask, sc * (DH ** -0.5), NEG)
            mx = jnp.max(sc, axis=1, keepdims=True)
            e = jnp.exp(sc - mx)
            den = jnp.sum(e, axis=1, keepdims=True)
            inv = pl.reciprocal(den, approx=True)
            inv = inv * (2.0 - den * inv)
            o = _dot(e.astype(bf16), va) * inv
            q_r[h][pl.ds(ra_, SEG), :] = o[MEM:]
            o_mem[h] = o[:MEM]

        def wo(g):
            hs = range(g * WO_GROUP, (g + 1) * WO_GROUP)
            lo = jnp.concatenate(
                [jnp.concatenate([o_mem.pop(h), q_r[h][pl.ds(rw_, TOK), :]], axis=0)
                 for h in hs], axis=1).astype(bf16)
            w = _unpack(wo_b[pl.ds(g * WO_GROUP * DH // 2, WO_GROUP * DH // 2), :])
            r = _dot(lo, w)
            total[0] = r if total[0] is None else total[0] + r

        if PAIRS:
            npair = H // 2
            t = 0
            nwo = 0
            while nwo < npair:
                for item in PATTERN:
                    if item == 'a' and t < npair:
                        qkv(2 * t)
                    if item == 'b' and t < npair:
                        qkv(2 * t + 1)
                    if item == 's':
                        if 0 <= t - LAG_QK < npair:
                            qk(2 * (t - LAG_QK))
                            qk(2 * (t - LAG_QK) + 1)
                        if 0 <= t - LAG_PV < npair:
                            pv(2 * (t - LAG_PV))
                            pv(2 * (t - LAG_PV) + 1)
                    if item == 'w' and 0 <= t - LAG_WO < npair:
                        wo(2 * (t - LAG_WO))
                        wo(2 * (t - LAG_WO) + 1)
                        nwo += 1
                    if item == 'f':
                        if t == F0_AT:
                            filler(0)
                        if t == F1_AT:
                            filler(1)
                t += 1
            if F1_AT < 0:
                filler(1)
        else:
            ng = H // WO_GROUP
            nxt = 0
            done_pv = 0
            t = 0
            while nxt < ng:
                if t < H:
                    qkv(t)
                if 0 <= t - LAG_QK < H:
                    qk(t - LAG_QK)
                if t == F0_AT:
                    filler(0)
                if t == F1_AT:
                    filler(1)
                if 0 <= t - LAG_PV < H:
                    pv(t - LAG_PV)
                    done_pv = t - LAG_PV + 1
                while (nxt < ng and t >= (nxt + 1) * WO_GROUP - 1 + LAG_WO
                       and done_pv >= (nxt + 1) * WO_GROUP):
                    wo(nxt)
                    nxt += 1
                t += 1
            if F1_AT < 0:
                filler(1)

        a = total[0]
        hr = pl.multiple_of(TOK * s, 8)
        hbuf[pl.ds(hr, TOK), :] += a[MEM:]
        return a[:MEM], wrap(rp + TOK), wrap(ra + SEG), wrap(rw + TOK)

    def steps(i, carry):
        if PROF > 1: scope('s06b_step')
        toks = [load_tok(i * UNROLL + k) for k in range(UNROLL)]
        for k in range(UNROLL):
            carry = step(i * UNROLL + k, carry, toks[k])
        if PROF > 1: scope(None)
        return carry

    scope('s06_loop')
    if not SKIP_LOOP: lax.fori_loop(
        0, NSEG // UNROLL, steps,
        (mem0_ref[...].astype(f32), jnp.int32(P0), jnp.int32(0), jnp.int32(0)))

    scope(None)
    def tail(yall, t0, t1, acc):
        scope('s07_post')
        if not SKIP_PRO:
            w2_copy.wait()
            w3_copy.wait()
            w4_copy.wait()
        if not SKIP_POST:

            def wo_batch(r0, n):
                rr = r0 % RING
                lo = jnp.concatenate(
                    [q_r[h][pl.ds(rr, n), :].astype(bf16) for h in range(H)], axis=1)
                hbuf[pl.ds(r0, n), :] += _dot(lo, _unpack(wo_b[...]))

            us = {}

            def mixer_u(r0, n):
                us[r0] = _ln(_ln(hbuf[pl.ds(r0, n), :])).astype(bf16)

            def mixer_in(r0, n):
                u = us.pop(r0)
                for c in range(4):
                    xg[c, pl.ds(HALO + r0, n), :] = _gelu(_dot(u, _unpack(w1b[c])))

            hss = {}

            def mixer_out(i):
                r0 = i * RB
                parts = []
                for c, off in enumerate((-1, 1, -2, 2)):
                    win = xg[c, pl.ds(r0, RB + 2 * HALO), :]
                    parts.append(win[HALO + off:HALO + off + RB].astype(bf16))
                if KCH:
                    hs = None
                    for c in range(4):
                        r = _dot(parts[c], _unpack(w2b[pl.ds(c * C4 // 2, C4 // 2), :]))
                        hs = r if hs is None else hs + r
                else:
                    hs = _dot(jnp.concatenate(parts, axis=1), _unpack(w2b[...]))
                hss[i] = hs

            def mixer_post(i):
                r0 = i * RB
                hv = hbuf[pl.ds(r0, RB), :]
                x1 = _ln(hv) + hss.pop(i)
                yall[pl.ds(r0 // 2, RB // 2), :] = _pack(_ln(x1))
                hbuf[pl.ds(r0, RB), :] = hv + x1

            done = TOK * NSEG
            split = 3 * RING
            first = 4 * TOK * (NSEG // 4 - 1)
            ops = {
                'A': lambda: wo_batch(done, split - done),
                'B': lambda: wo_batch(split, S - split),
                't': lambda: mixer_u(first, done - first),
                'T': lambda: mixer_in(first, done - first),
                'u': lambda: mixer_u(done, split - done),
                'U': lambda: mixer_in(done, split - done),
                'r': lambda: mixer_u(first, split - first),
                'R': lambda: mixer_in(first, split - first),
                'v': lambda: mixer_u(split, S - split),
                'V': lambda: mixer_in(split, S - split),
            }
            for i in range(S // RB):
                ops[str(i)] = functools.partial(mixer_out, i)
                ops[chr(ord('a') + i)] = functools.partial(mixer_post, i)
            for ch in POSTORD:
                ops[ch]()

        scope('s08_mlp')
        ts = (t0, t1)
        nc = F // FC

        def mlp_block(i, carry):
            rows = pl.ds(pl.multiple_of(i * RB, RB), RB)

            def up(c):
                y = _unpack(yall[pl.ds(pl.multiple_of(i * (RB // 2), RB // 2), RB // 2), :])
                r = _dot(y, _unpack(w3b[:, c * FC:(c + 1) * FC]))
                ts[c % 2][...] = _pack(_gelu(r))

            def down(c):
                r = _dot(_unpack(ts[c % 2][...]),
                         _unpack(w4b[c * FC // 2:(c + 1) * FC // 2, :]))
                if c == 0:
                    acc[...] = hbuf[rows, :] + r
                elif c < nc - 1:
                    acc[...] += r
                else:
                    xs[rows, :] = (acc[...] + r).astype(bf16)

            up(0)
            for c in range(nc):
                if c + 1 < nc:
                    up(c + 1)
                down(c)
            out_copy(i).start()
            return carry

        if not SKIP_MLP:
            lax.fori_loop(0, S // RB, mlp_block, 0)
            scope('s09_outwait')
            for i in range(S // RB):
                out_copy(i).wait()
        scope(None)

    pl.run_scoped(
        tail,
        pltpu.VMEM((S // 2, D), u32),
        pltpu.VMEM((RB // 2, FC), u32),
        pltpu.VMEM((RB // 2, FC), u32),
        pltpu.VMEM((RB, D), f32),
    )


@jax.jit
def pallas_sequential_preLN__memory_aug_recurrent_mem_tr__mixer_s_mlp__prompt_kernel(
    A_x: jax.Array,
    A_mem0: jax.Array,
    A_Wq: jax.Array,
    A_Wk: jax.Array,
    A_Wv: jax.Array,
    A_Wo: jax.Array,
    A_seg_len: jax.Array,
    B_x: jax.Array,
    B_w1: jax.Array,
    B_w2: jax.Array,
    B_w3: jax.Array,
    B_w4: jax.Array,
):
    del A_seg_len, B_x
    hbm = pl.BlockSpec(memory_space=pl.ANY)
    vmem = pl.BlockSpec(memory_space=pltpu.VMEM)
    scratch = [
        pltpu.VMEM((H, D // 2, DH), u32),
        pltpu.VMEM((H, D // 2, DH), u32),
        pltpu.VMEM((H, D // 2, DH), u32),
        pltpu.VMEM((H * DH // 2, D), u32),
        pltpu.VMEM((S, D), bf16),
        pltpu.VMEM((S, D), f32),
        pltpu.VMEM((4, S + 2 * HALO, C4), f32),
        pltpu.VMEM((2 * TOK, D), u32),
        pltpu.VMEM((4, D // 2, C4), u32),
        pltpu.VMEM((D // 2, D), u32),
        pltpu.VMEM((D // 2, F), u32),
        pltpu.VMEM((F // 2, D), u32),
        pltpu.SemaphoreType.DMA((48,)),
    ] + [pltpu.VMEM((H // 8, RING, DH), f32)] * 24
    out = pl.pallas_call(
        _kernel,
        out_shape=jax.ShapeDtypeStruct((S, D), A_x.dtype),
        in_specs=[hbm, vmem] + [hbm] * 8,
        out_specs=hbm,
        scratch_shapes=scratch,
        compiler_params=pltpu.CompilerParams(vmem_limit_bytes=126 * 1024 * 1024),
    )(A_x.reshape(S, D), A_mem0.reshape(MEM, D),
      A_Wq.reshape(D // 2, 2 * H, DH), A_Wk.reshape(D // 2, 2 * H, DH),
      A_Wv.reshape(D // 2, 2 * H, DH),
      A_Wo.reshape(H * DH, D), B_w1, B_w2, B_w3, B_w4)
    return out.reshape(A_x.shape)
```

```python
import functools

import jax
import jax.numpy as jnp
from jax import lax
import jax.experimental.pallas as pl
import jax.experimental.pallas.tpu as pltpu

S = 2048
D = 1024
H = 32
DH = 128
MEM = 8
SEG = 32
F = 3584
NSEG = S // SEG
L = MEM + SEG
TOK = 24
P0 = S - TOK * NSEG
RING = 576
C4 = D // 4
HALO = 8
RB = 256
FC = 512
EPS = 1e-5
NEG = -1000000000.0

bf16 = jnp.bfloat16
f32 = jnp.float32
u32 = jnp.uint32

LAG_QK = 2
LAG_PV = 4
LAG_WO = 6
WO_GROUP = 1
import os as _os
_env = lambda k, d: int(_os.environ.get(k, d))
UNROLL = _env('UNROLL', 2)
LAG_QK = _env('LAG_QK', LAG_QK); LAG_PV = _env('LAG_PV', LAG_PV); LAG_WO = _env('LAG_WO', LAG_WO); WO_GROUP = _env('WO_GROUP', WO_GROUP)
SKIP_PRO = _env('SKIP_PRO', 0); SKIP_POST = _env('SKIP_POST', 0); SKIP_LOOP = _env('SKIP_LOOP', 0); SKIP_MLP = _env('SKIP_MLP', 0)
PAIRS = _env('PAIRS', 1)
PATTERN = _os.environ.get('PATTERN', 'sabfw')
KCH = _env('KCH', 1)
POSTORD = _os.environ.get('POSTORD', 'tATuBU01v2aVb3c45d6e7fgh')
STG3 = _env('STG3', 1)
STW = _env('STW', 0)
PMAJ = _env('PMAJ', 0)
NI = _env('NI', 8)
RELAY_SPAN = _env('RELAY_SPAN', 8)
WAIT_AT = _env('WAIT_AT', 5)
import contextlib
PROF = _env('PROF', 0)
class _Scopes:
    cur = None
    def __call__(self, name):
        if not PROF: return
        if self.cur is not None: self.cur.__exit__(None, None, None)
        self.cur = None
        if name is not None:
            self.cur = jax.named_scope(name); self.cur.__enter__()
F0_AT = _env('F0_AT', 18); F1_AT = _env('F1_AT', -1)


def mult(i, n):
    return i if isinstance(i, int) else pl.multiple_of(i, n)


def _ln(x):
    m = jnp.mean(x, axis=-1, keepdims=True)
    d = x - m
    v = jnp.mean(d * d, axis=-1, keepdims=True)
    return d * lax.rsqrt(v + EPS)


def _gelu(x):
    return jax.nn.gelu(x, approximate=True)


def _pack(x):
    return pltpu.bitcast(x.astype(bf16), u32)


def _unpack(x):
    return pltpu.bitcast(x, bf16)


def _dot(a, b):
    return jnp.dot(a, b, preferred_element_type=f32)


def _kernel(x_hbm, mem0_ref, wq_hbm, wk_hbm, wv_hbm, wo_hbm, w1_hbm, w2_hbm,
            w3_hbm, w4_hbm, out_hbm,
            wq_s, wk_s, wv_s, wo_b, xs, hbuf, xg, ubuf,
            w1b, w2b, w3b, w4b, sems, *rings):
    scope = _Scopes()
    w_hbm = (wq_hbm, wk_hbm, wv_hbm)
    w_s = (wq_s, wk_s, wv_s)
    ring = [[rings[m * 8 + h % 8].at[h // 8] for h in range(H)] for m in range(3)]
    q_r, k_r, v_r = ring

    SEM_X0, SEM_X, SEM_WO, SEM_W1, SEM_W2, SEM_W3, SEM_W4, SEM_OUT, SEM_W = (
        0, 1, 13, 21, 25, 26, 27, 28, 36)
    XP = (S - P0) // 12

    x0_copy = pltpu.make_async_copy(x_hbm.at[pl.ds(0, P0)], xs.at[pl.ds(0, P0)],
                                    sems.at[SEM_X0])

    def x_copy(g):
        rows = pl.ds(mult(P0 + g * 3 * XP, XP), 3 * XP)
        return pltpu.make_async_copy(x_hbm.at[rows], xs.at[rows], sems.at[SEM_X + g])

    def wo_copy(i):
        rows = pl.ds(mult(i * 512, 512), 512)
        return pltpu.make_async_copy(wo_hbm.bitcast(u32).at[rows], wo_b.at[rows],
                                     sems.at[SEM_WO + i])

    def w1_copy(i):
        cols = pl.ds(mult(i * C4, C4), C4)
        return pltpu.make_async_copy(w1_hbm.bitcast(u32).at[:, cols], w1b.at[i],
                                     sems.at[SEM_W1 + i])

    w2_copy = pltpu.make_async_copy(w2_hbm.bitcast(u32), w2b, sems.at[SEM_W2])
    w3_copy = pltpu.make_async_copy(w3_hbm.bitcast(u32), w3b, sems.at[SEM_W3])
    w4_copy = pltpu.make_async_copy(w4_hbm.bitcast(u32), w4b, sems.at[SEM_W4])

    def out_copy(i):
        rows = pl.ds(pl.multiple_of(i * RB, RB), RB)
        return pltpu.make_async_copy(xs.at[rows], out_hbm.at[rows], sems.at[SEM_OUT + i])

    def prologue(stg0, stg1, stg2, lhs0):
        stg = (stg0, stg1, stg2)

        def w_copies(g, m):
            src = w_hbm[m].bitcast(u32)
            dst = stg[m].reshape(D // 2, 8, DH)
            return [pltpu.make_async_copy(
                src.at[:, pl.ds(pl.multiple_of(16 * par + 4 * g, 4), 4), :],
                dst.at[:, pl.ds(4 * par, 4), :],
                sems.at[SEM_W + 3 * g + m]) for par in range(2)]

        def start(copies):
            for cp in copies:
                cp.start()

        def wait(copies):
            for cp in copies:
                cp.wait()

        def relayout(g, m, pair, i0, n):
            ev = stg[m][pl.ds(8 * i0 + pair, n, stride=8), :]
            od = stg[m][pl.ds(8 * i0 + 4 + pair, n, stride=8), :]
            h = 8 * g + 2 * pair
            w_s[m][h, pl.ds(i0, n), :] = (ev & jnp.uint32(0xFFFF)) | (od << 16)
            w_s[m][h + 1, pl.ds(i0, n), :] = (ev >> 16) | (od & jnp.uint32(0xFFFF0000))

        def norm_rows(r0, n, to_lhs0):
            xv = xs[pl.ds(r0, n), :].astype(f32)
            hbuf[pl.ds(r0, n), :] = xv
            xn = _ln(xv)
            if to_lhs0:
                lhs0[pl.ds(pl.multiple_of(r0 // 2, n // 2), n // 2), :] = _pack(xn)
            else:
                for c in range(4):
                    xg[c, pl.ds(HALO + r0, n), :] = xn[:, c * C4:(c + 1) * C4]

        scope('s00_init')
        x0_copy.start()
        start(w_copies(0, 0))
        start(w_copies(0, 1))
        x_copy(0).start()
        start(w_copies(0, 2))
        w1_copy(0).start()
        zero = jnp.zeros((HALO, C4), f32)
        for c in range(4):
            xg[c, pl.ds(0, HALO), :] = zero
            xg[c, pl.ds(HALO + S, HALO), :] = zero
        x0_copy.wait()
        scope('s01_norm0')

        @pl.loop(0, P0 // 128)
        def _(i):
            norm_rows(pl.multiple_of(i * 128, 128), 128, True)

        scope('s02_waitw0')
        pltpu.make_async_copy(stg[0], stg[0], sems.at[SEM_W]).wait()
        scope('s03_rel0')

        @pl.loop(0, 4)
        def _(pair):
            for i0 in range(0, D // 2, 64):
                relayout(0, 0, pair, i0, 64)


        def stage(c, g, m):
            m1 = (m + 1) % 3
            g1 = jnp.minimum(g + (1 if m == 2 else 0), 3)
            pieces = ([(pair, i0) for pair in range(4) for i0 in range(0, D // 2, NI)] if PMAJ else
                      [(pair, i0) for i0 in range(0, D // 2, NI) for pair in range(4)])
            span = 8 - WAIT_AT
            cuts = [len(pieces) * k // span for k in range(span + 1)]
            rcuts = [XP // 16 * k // span * 16 for k in range(span + 1)]

            def waits():
                @pl.when(c < 11)
                def _():
                    pltpu.make_async_copy(stg[m1], stg[m1],
                                          sems.at[SEM_W + 3 * g1 + m1]).wait()
                if m == 0:
                    x_copy(g).wait()

            def starts():
                @pl.when(g < 3)
                def _():
                    start(w_copies(g + 1, m))
                    if m == 0:
                        x_copy(g + 1).start()
                    if m == 2:
                        w1_copy(g + 1).start()
                if m == 1:
                    wo_copy(g).start()

            for j in range(8):
                if j >= WAIT_AT:
                    k = j - WAIT_AT
                    for pair, i0 in pieces[cuts[k]:cuts[k + 1]]:
                        relayout(g1, m1, pair, i0, NI)
                    nr = rcuts[k + 1] - rcuts[k]
                    if nr:
                        norm_rows(pl.multiple_of(P0 + c * XP + rcuts[k], 16), nr, False)
                res = _dot(_unpack(lhs0[...]), _unpack(w_s[m][8 * g + j]))
                if j == WAIT_AT - 1:
                    if STW:
                        starts()
                    waits()
                if j == 7 and not STW:
                    starts()
                rings[m * 8 + j][g, pl.ds(0, P0), :] = res

        def stages(c, carry):
            g = c // 3
            if PROF > 1: scope('s04b_stage')
            for m in range(3):
                pl.when(c - 3 * g == m)(functools.partial(stage, c, g, m))
            if PROF > 1: scope(None)
            return carry

        def stages3(g, carry):
            for m in range(3):
                stage(3 * g + m, g, m)
            return carry

        scope('s04_stages')
        if STG3:
            lax.fori_loop(0, 4, stages3, 0)
        else:
            lax.fori_loop(0, 12, stages, 0)
        scope(None)

    if not SKIP_PRO:
        pl.run_scoped(
            prologue,
            pltpu.VMEM((8 * D // 2, DH), u32),
            pltpu.VMEM((8 * D // 2, DH), u32),
            pltpu.VMEM((8 * D // 2, DH), u32),
            pltpu.VMEM((P0 // 2, D), u32),
        )
        scope('s05_waitwo')
        w2_copy.start()
        w3_copy.start()
        w4_copy.start()
        for i in range(4):
            wo_copy(i).wait()
        for i in range(4):
            w1_copy(i).wait()

    def wrap(r):
        return jnp.where(r >= RING, r - RING, r)

    def load_tok(s):
        t_tok = pl.multiple_of(HALO + P0 + TOK * s, 8)
        return jnp.concatenate([xg[c, pl.ds(t_tok, TOK), :] for c in range(4)], axis=1)

    def step(s, carry, tok):
        mem, rp, ra, rw = carry

        ri = lax.broadcasted_iota(jnp.int32, (L, L), 0)
        ci = lax.broadcasted_iota(jnp.int32, (L, L), 1)
        mask = (ri < MEM) | (ri >= ci)

        lhs = jnp.concatenate([mem, tok], axis=0).astype(bf16)
        rps = [pl.multiple_of(wrap(rp + 8 * i), 8) for i in range(3)]
        ra_ = pl.multiple_of(ra, SEG)
        rw_ = pl.multiple_of(rw, 8)

        col = s & 3
        rb = pl.multiple_of(jnp.maximum((s >> 2) - 1, 0) * (4 * TOK), 8)
        ubuf[...] = _pack(_ln(_ln(hbuf[pl.ds(rb, 4 * TOK), :])))

        def filler(j):
            u = _unpack(ubuf[...])
            r = _dot(u, _unpack(w1b[col, :, pl.ds(j * 128, 128)]))
            xg[col, pl.ds(HALO + rb, 4 * TOK), pl.ds(j * 128, 128)] = _gelu(r)

        mem_qkv = {}
        scores = {}
        o_mem = {}
        total = [None]

        def qkv(h):
            res = []
            for m in range(3):
                r = _dot(lhs, _unpack(w_s[m][h]))
                for i in range(3):
                    ring[m][h][pl.ds(rps[i], 8), :] = r[8 + 8 * i:16 + 8 * i]
                res.append(r[:MEM])
            mem_qkv[h] = res

        def qk(h):
            qm, km, vm = mem_qkv.pop(h)
            qa = jnp.concatenate([qm, q_r[h][pl.ds(ra_, SEG), :]], axis=0).astype(bf16)
            ka = jnp.concatenate([km, k_r[h][pl.ds(ra_, SEG), :]], axis=0).astype(bf16)
            sc = lax.dot_general(qa, ka, (((1,), (1,)), ((), ())),
                                 preferred_element_type=f32)
            scores[h] = (sc, vm)

        def pv(h):
            sc, vm = scores.pop(h)
            va = jnp.concatenate([vm, v_r[h][pl.ds(ra_, SEG), :]], axis=0).astype(bf16)
            sc = jnp.where(mask, sc * (DH ** -0.5), NEG)
            mx = jnp.max(sc, axis=1, keepdims=True)
            e = jnp.exp(sc - mx)
            den = jnp.sum(e, axis=1, keepdims=True)
            inv = pl.reciprocal(den, approx=True)
            inv = inv * (2.0 - den * inv)
            o = _dot(e.astype(bf16), va) * inv
            q_r[h][pl.ds(ra_, SEG), :] = o[MEM:]
            o_mem[h] = o[:MEM]

        def wo(g):
            hs = range(g * WO_GROUP, (g + 1) * WO_GROUP)
            lo = jnp.concatenate(
                [jnp.concatenate([o_mem.pop(h), q_r[h][pl.ds(rw_, TOK), :]], axis=0)
                 for h in hs], axis=1).astype(bf16)
            w = _unpack(wo_b[pl.ds(g * WO_GROUP * DH // 2, WO_GROUP * DH // 2), :])
            r = _dot(lo, w)
            total[0] = r if total[0] is None else total[0] + r

        if PAIRS:
            npair = H // 2
            t = 0
            nwo = 0
            while nwo < npair:
                for item in PATTERN:
                    if item == 'a' and t < npair:
                        qkv(2 * t)
                    if item == 'b' and t < npair:
                        qkv(2 * t + 1)
                    if item == 's':
                        if 0 <= t - LAG_QK < npair:
                            qk(2 * (t - LAG_QK))
                            qk(2 * (t - LAG_QK) + 1)
                        if 0 <= t - LAG_PV < npair:
                            pv(2 * (t - LAG_PV))
                            pv(2 * (t - LAG_PV) + 1)
                    if item == 'w' and 0 <= t - LAG_WO < npair:
                        wo(2 * (t - LAG_WO))
                        wo(2 * (t - LAG_WO) + 1)
                        nwo += 1
                    if item == 'f':
                        if t == F0_AT:
                            filler(0)
                        if t == F1_AT:
                            filler(1)
                t += 1
            if F1_AT < 0:
                filler(1)
        else:
            ng = H // WO_GROUP
            nxt = 0
            done_pv = 0
            t = 0
            while nxt < ng:
                if t < H:
                    qkv(t)
                if 0 <= t - LAG_QK < H:
                    qk(t - LAG_QK)
                if t == F0_AT:
                    filler(0)
                if t == F1_AT:
                    filler(1)
                if 0 <= t - LAG_PV < H:
                    pv(t - LAG_PV)
                    done_pv = t - LAG_PV + 1
                while (nxt < ng and t >= (nxt + 1) * WO_GROUP - 1 + LAG_WO
                       and done_pv >= (nxt + 1) * WO_GROUP):
                    wo(nxt)
                    nxt += 1
                t += 1
            if F1_AT < 0:
                filler(1)

        a = total[0]
        hr = pl.multiple_of(TOK * s, 8)
        hbuf[pl.ds(hr, TOK), :] += a[MEM:]
        return a[:MEM], wrap(rp + TOK), wrap(ra + SEG), wrap(rw + TOK)

    def steps(i, carry):
        if PROF > 1: scope('s06b_step')
        toks = [load_tok(i * UNROLL + k) for k in range(UNROLL)]
        for k in range(UNROLL):
            carry = step(i * UNROLL + k, carry, toks[k])
        if PROF > 1: scope(None)
        return carry

    scope('s06_loop')
    if not SKIP_LOOP: lax.fori_loop(
        0, NSEG // UNROLL, steps,
        (mem0_ref[...].astype(f32), jnp.int32(P0), jnp.int32(0), jnp.int32(0)))

    scope(None)
    def tail(yall, t0, t1, acc):
        scope('s07_post')
        if not SKIP_PRO:
            w2_copy.wait()
            w3_copy.wait()
            w4_copy.wait()
        if not SKIP_POST:

            def wo_batch(r0, n):
                rr = r0 % RING
                lo = jnp.concatenate(
                    [q_r[h][pl.ds(rr, n), :].astype(bf16) for h in range(H)], axis=1)
                hbuf[pl.ds(r0, n), :] += _dot(lo, _unpack(wo_b[...]))

            us = {}

            def mixer_u(r0, n):
                us[r0] = _ln(_ln(hbuf[pl.ds(r0, n), :])).astype(bf16)

            def mixer_in(r0, n):
                u = us.pop(r0)
                for c in range(4):
                    xg[c, pl.ds(HALO + r0, n), :] = _gelu(_dot(u, _unpack(w1b[c])))

            hss = {}

            def mixer_out(i):
                r0 = i * RB
                parts = []
                for c, off in enumerate((-1, 1, -2, 2)):
                    win = xg[c, pl.ds(r0, RB + 2 * HALO), :]
                    parts.append(win[HALO + off:HALO + off + RB].astype(bf16))
                if KCH:
                    hs = None
                    for c in range(4):
                        r = _dot(parts[c], _unpack(w2b[pl.ds(c * C4 // 2, C4 // 2), :]))
                        hs = r if hs is None else hs + r
                else:
                    hs = _dot(jnp.concatenate(parts, axis=1), _unpack(w2b[...]))
                hss[i] = hs

            def mixer_post(i):
                r0 = i * RB
                hv = hbuf[pl.ds(r0, RB), :]
                x1 = _ln(hv) + hss.pop(i)
                yall[pl.ds(r0 // 2, RB // 2), :] = _pack(_ln(x1))
                hbuf[pl.ds(r0, RB), :] = hv + x1

            done = TOK * NSEG
            split = 3 * RING
            first = 4 * TOK * (NSEG // 4 - 1)
            ops = {
                'A': lambda: wo_batch(done, split - done),
                'B': lambda: wo_batch(split, S - split),
                'P': lambda: wo_batch(done, 96),
                'Q': lambda: wo_batch(done + 96, 96),
                'X': lambda: wo_batch(split, 160),
                'Y': lambda: wo_batch(split + 160, 160),
                'x': lambda: mixer_u(split, 160),
                'y': lambda: mixer_u(split + 160, 160),
                'M': lambda: mixer_in(split, 160),
                'N': lambda: mixer_in(split + 160, 160),
                't': lambda: mixer_u(first, done - first),
                'T': lambda: mixer_in(first, done - first),
                'u': lambda: mixer_u(done, split - done),
                'U': lambda: mixer_in(done, split - done),
                'r': lambda: mixer_u(first, split - first),
                'R': lambda: mixer_in(first, split - first),
                'v': lambda: mixer_u(split, S - split),
                'V': lambda: mixer_in(split, S - split),
            }
            for i in range(S // RB):
                ops[str(i)] = functools.partial(mixer_out, i)
                ops[chr(ord('a') + i)] = functools.partial(mixer_post, i)
            for ch in POSTORD:
                ops[ch]()

        scope('s08_mlp')
        ts = (t0, t1)
        nc = F // FC

        def mlp_block(i, carry):
            rows = pl.ds(pl.multiple_of(i * RB, RB), RB)

            def up(c):
                y = _unpack(yall[pl.ds(pl.multiple_of(i * (RB // 2), RB // 2), RB // 2), :])
                r = _dot(y, _unpack(w3b[:, c * FC:(c + 1) * FC]))
                ts[c % 2][...] = _pack(_gelu(r))

            def down(c):
                r = _dot(_unpack(ts[c % 2][...]),
                         _unpack(w4b[c * FC // 2:(c + 1) * FC // 2, :]))
                if c == 0:
                    acc[...] = hbuf[rows, :] + r
                elif c < nc - 1:
                    acc[...] += r
                else:
                    xs[rows, :] = (acc[...] + r).astype(bf16)

            up(0)
            for c in range(nc):
                if c + 1 < nc:
                    up(c + 1)
                down(c)
            out_copy(i).start()
            return carry

        if not SKIP_MLP:
            lax.fori_loop(0, S // RB, mlp_block, 0)
            scope('s09_outwait')
            for i in range(S // RB):
                out_copy(i).wait()
        scope(None)

    pl.run_scoped(
        tail,
        pltpu.VMEM((S // 2, D), u32),
        pltpu.VMEM((RB // 2, FC), u32),
        pltpu.VMEM((RB // 2, FC), u32),
        pltpu.VMEM((RB, D), f32),
    )


@jax.jit
def pallas_sequential_preLN__memory_aug_recurrent_mem_tr__mixer_s_mlp__prompt_kernel(
    A_x: jax.Array,
    A_mem0: jax.Array,
    A_Wq: jax.Array,
    A_Wk: jax.Array,
    A_Wv: jax.Array,
    A_Wo: jax.Array,
    A_seg_len: jax.Array,
    B_x: jax.Array,
    B_w1: jax.Array,
    B_w2: jax.Array,
    B_w3: jax.Array,
    B_w4: jax.Array,
):
    del A_seg_len, B_x
    hbm = pl.BlockSpec(memory_space=pl.ANY)
    vmem = pl.BlockSpec(memory_space=pltpu.VMEM)
    scratch = [
        pltpu.VMEM((H, D // 2, DH), u32),
        pltpu.VMEM((H, D // 2, DH), u32),
        pltpu.VMEM((H, D // 2, DH), u32),
        pltpu.VMEM((H * DH // 2, D), u32),
        pltpu.VMEM((S, D), bf16),
        pltpu.VMEM((S, D), f32),
        pltpu.VMEM((4, S + 2 * HALO, C4), f32),
        pltpu.VMEM((2 * TOK, D), u32),
        pltpu.VMEM((4, D // 2, C4), u32),
        pltpu.VMEM((D // 2, D), u32),
        pltpu.VMEM((D // 2, F), u32),
        pltpu.VMEM((F // 2, D), u32),
        pltpu.SemaphoreType.DMA((48,)),
    ] + [pltpu.VMEM((H // 8, RING, DH), f32)] * 24
    out = pl.pallas_call(
        _kernel,
        out_shape=jax.ShapeDtypeStruct((S, D), A_x.dtype),
        in_specs=[hbm, vmem] + [hbm] * 8,
        out_specs=hbm,
        scratch_shapes=scratch,
        compiler_params=pltpu.CompilerParams(vmem_limit_bytes=126 * 1024 * 1024),
    )(A_x.reshape(S, D), A_mem0.reshape(MEM, D),
      A_Wq.reshape(D // 2, 2 * H, DH), A_Wk.reshape(D // 2, 2 * H, DH),
      A_Wv.reshape(D // 2, 2 * H, DH),
      A_Wo.reshape(H * DH, D), B_w1, B_w2, B_w3, B_w4)
    return out.reshape(A_x.shape)
```

```python
import functools

import jax
import jax.numpy as jnp
from jax import lax
import jax.experimental.pallas as pl
import jax.experimental.pallas.tpu as pltpu

S = 2048
D = 1024
H = 32
DH = 128
MEM = 8
SEG = 32
F = 3584
NSEG = S // SEG
L = MEM + SEG
TOK = 24
P0 = S - TOK * NSEG
RING = 576
XP = (S - P0) // 12
C4 = D // 4
HALO = 8
RB = 256
FC = 512
EPS = 1e-5
NEG = -1000000000.0

LAG_QK, LAG_PV, LAG_WO = 2, 4, 6
FILL_AT = 18
UNROLL = 2

bf16 = jnp.bfloat16
f32 = jnp.float32
u32 = jnp.uint32

SEM_X0, SEM_X, SEM_WO, SEM_W1, SEM_W2, SEM_W3, SEM_W4, SEM_OUT, SEM_W = (
    0, 1, 5, 9, 13, 14, 15, 16, 32)
NSEM = SEM_W + 12


def _mult(i, n):
    return i if isinstance(i, int) else pl.multiple_of(i, n)


def _ln(x):
    m = jnp.mean(x, axis=-1, keepdims=True)
    d = x - m
    v = jnp.mean(d * d, axis=-1, keepdims=True)
    return d * lax.rsqrt(v + EPS)


def _gelu(x):
    return jax.nn.gelu(x, approximate=True)


def _pack(x):
    return pltpu.bitcast(x.astype(bf16), u32)


def _unpack(x):
    return pltpu.bitcast(x, bf16)


def _dot(a, b):
    return jnp.dot(a, b, preferred_element_type=f32)


def _kernel(x_hbm, mem0_ref, wq_hbm, wk_hbm, wv_hbm, wo_hbm, w1_hbm, w2_hbm,
            w3_hbm, w4_hbm, out_hbm,
            wq_s, wk_s, wv_s, wo_b, xs, hbuf, xg, ubuf,
            w1b, w2b, w3b, w4b, sems, *rings):
    w_hbm = (wq_hbm, wk_hbm, wv_hbm)
    w_s = (wq_s, wk_s, wv_s)
    ring = [[rings[m * 8 + h % 8].at[h // 8] for h in range(H)] for m in range(3)]
    q_r, k_r, v_r = ring

    x0_copy = pltpu.make_async_copy(x_hbm.at[pl.ds(0, P0)], xs.at[pl.ds(0, P0)],
                                    sems.at[SEM_X0])

    def x_copy(g):
        rows = pl.ds(_mult(P0 + g * 3 * XP, XP), 3 * XP)
        return pltpu.make_async_copy(x_hbm.at[rows], xs.at[rows], sems.at[SEM_X + g])

    def wo_copy(i):
        rows = pl.ds(_mult(i * 512, 512), 512)
        return pltpu.make_async_copy(wo_hbm.bitcast(u32).at[rows], wo_b.at[rows],
                                     sems.at[SEM_WO + i])

    def w1_copy(i):
        cols = pl.ds(_mult(i * C4, C4), C4)
        return pltpu.make_async_copy(w1_hbm.bitcast(u32).at[:, cols], w1b.at[i],
                                     sems.at[SEM_W1 + i])

    w2_copy = pltpu.make_async_copy(w2_hbm.bitcast(u32), w2b, sems.at[SEM_W2])
    w3_copy = pltpu.make_async_copy(w3_hbm.bitcast(u32), w3b, sems.at[SEM_W3])
    w4_copy = pltpu.make_async_copy(w4_hbm.bitcast(u32), w4b, sems.at[SEM_W4])

    def out_copy(i):
        rows = pl.ds(_mult(i * (RB // 2), RB // 2), RB // 2)
        return pltpu.make_async_copy(xs.at[rows], out_hbm.at[rows], sems.at[SEM_OUT + i])

    def prologue(stg0, stg1, stg2, lhs0):
        stg = (stg0, stg1, stg2)

        def start_chunk(g, m):
            src = w_hbm[m].bitcast(u32)
            dst = stg[m].reshape(D // 2, 8, DH)
            for par in range(2):
                pltpu.make_async_copy(
                    src.at[:, pl.ds(_mult(16 * par + 4 * g, 4), 4), :],
                    dst.at[:, pl.ds(4 * par, 4), :],
                    sems.at[SEM_W + 3 * g + m]).start()

        def wait_chunk(g, m):
            pltpu.make_async_copy(stg[m], stg[m], sems.at[SEM_W + 3 * g + m]).wait()

        def relayout(g, m, pair, i0, n):
            ev = stg[m][pl.ds(8 * i0 + pair, n, stride=8), :]
            od = stg[m][pl.ds(8 * i0 + 4 + pair, n, stride=8), :]
            h = 8 * g + 2 * pair
            w_s[m][h, pl.ds(i0, n), :] = (ev & jnp.uint32(0xFFFF)) | (od << 16)
            w_s[m][h + 1, pl.ds(i0, n), :] = (ev >> 16) | (od & jnp.uint32(0xFFFF0000))

        def norm_rows(r0, n, to_lhs0):
            xv = xs[pl.ds(r0, n), :].astype(f32)
            hbuf[pl.ds(r0, n), :] = xv
            xn = _ln(xv)
            if to_lhs0:
                lhs0[pl.ds(pl.multiple_of(r0 // 2, n // 2), n // 2), :] = _pack(xn)
            else:
                for c in range(4):
                    xg[c, pl.ds(HALO + r0, n), :] = xn[:, c * C4:(c + 1) * C4]

        x0_copy.start()
        start_chunk(0, 0)
        start_chunk(0, 1)
        x_copy(0).start()
        start_chunk(0, 2)
        w1_copy(0).start()
        zero = jnp.zeros((HALO, C4), f32)
        for c in range(4):
            xg[c, pl.ds(0, HALO), :] = zero
            xg[c, pl.ds(HALO + S, HALO), :] = zero
        x0_copy.wait()

        @pl.loop(0, P0 // 128)
        def _(i):
            norm_rows(pl.multiple_of(i * 128, 128), 128, True)

        wait_chunk(0, 0)

        @pl.loop(0, 4)
        def _(pair):
            for i0 in range(0, D // 2, 64):
                relayout(0, 0, pair, i0, 64)

        def stage(g, m):
            c = 3 * g + m
            m1 = (m + 1) % 3
            g1 = jnp.minimum(g + (1 if m == 2 else 0), 3)
            pieces = [(pair, i0) for i0 in range(0, D // 2, 8) for pair in range(4)]
            wait_at = 5
            span = 8 - wait_at
            cuts = [len(pieces) * k // span for k in range(span + 1)]
            rcuts = [XP // 16 * k // span * 16 for k in range(span + 1)]
            for j in range(8):
                if j >= wait_at:
                    k = j - wait_at
                    for pair, i0 in pieces[cuts[k]:cuts[k + 1]]:
                        relayout(g1, m1, pair, i0, 8)
                    norm_rows(pl.multiple_of(P0 + c * XP + rcuts[k], 16),
                              rcuts[k + 1] - rcuts[k], False)
                res = _dot(_unpack(lhs0[...]), _unpack(w_s[m][8 * g + j]))
                if j == wait_at - 1:
                    pl.when(c < 11)(functools.partial(wait_chunk, g1, m1))
                    if m == 0:
                        x_copy(g).wait()
                if j == 7:
                    @pl.when(g < 3)
                    def _():
                        start_chunk(g + 1, m)
                        if m == 0:
                            x_copy(g + 1).start()
                        if m == 2:
                            w1_copy(g + 1).start()
                    if m == 1:
                        wo_copy(g).start()
                rings[m * 8 + j][g, pl.ds(0, P0), :] = res

        @pl.loop(0, 4)
        def _(g):
            for m in range(3):
                stage(g, m)

    pl.run_scoped(
        prologue,
        pltpu.VMEM((8 * D // 2, DH), u32),
        pltpu.VMEM((8 * D // 2, DH), u32),
        pltpu.VMEM((8 * D // 2, DH), u32),
        pltpu.VMEM((P0 // 2, D), u32),
    )
    w2_copy.start()
    w3_copy.start()
    w4_copy.start()
    for i in range(4):
        wo_copy(i).wait()
    for i in range(4):
        w1_copy(i).wait()

    def wrap(r):
        return jnp.where(r >= RING, r - RING, r)

    def load_tok(s):
        rows = pl.ds(pl.multiple_of(HALO + P0 + TOK * s, 8), TOK)
        return jnp.concatenate([xg[c, rows, :] for c in range(4)], axis=1)

    def step(s, carry, tok):
        mem, rp, ra, rw = carry
        ri = lax.broadcasted_iota(jnp.int32, (L, L), 0)
        ci = lax.broadcasted_iota(jnp.int32, (L, L), 1)
        mask = (ri < MEM) | (ri >= ci)

        lhs = jnp.concatenate([mem, tok], axis=0).astype(bf16)
        rps = [pl.multiple_of(wrap(rp + 8 * i), 8) for i in range(3)]
        ra_ = pl.multiple_of(ra, SEG)
        rw_ = pl.multiple_of(rw, 8)

        col = s & 3
        rb = pl.multiple_of(jnp.maximum((s >> 2) - 1, 0) * (4 * TOK), 8)
        ubuf[...] = _pack(_ln(_ln(hbuf[pl.ds(rb, 4 * TOK), :])))

        def filler(j):
            r = _dot(_unpack(ubuf[...]), _unpack(w1b[col, :, pl.ds(j * 128, 128)]))
            xg[col, pl.ds(HALO + rb, 4 * TOK), pl.ds(j * 128, 128)] = _gelu(r)

        mem_qkv = {}
        scores = {}
        o_mem = {}
        total = [None]

        def qkv(h):
            res = []
            for m in range(3):
                r = _dot(lhs, _unpack(w_s[m][h]))
                for i in range(3):
                    ring[m][h][pl.ds(rps[i], 8), :] = r[8 + 8 * i:16 + 8 * i]
                res.append(r[:MEM])
            mem_qkv[h] = res

        def qk(h):
            qm, km, vm = mem_qkv.pop(h)
            qa = jnp.concatenate([qm, q_r[h][pl.ds(ra_, SEG), :]], axis=0).astype(bf16)
            ka = jnp.concatenate([km, k_r[h][pl.ds(ra_, SEG), :]], axis=0).astype(bf16)
            sc = lax.dot_general(qa, ka, (((1,), (1,)), ((), ())),
                                 preferred_element_type=f32)
            scores[h] = (sc, vm)

        def pv(h):
            sc, vm = scores.pop(h)
            va = jnp.concatenate([vm, v_r[h][pl.ds(ra_, SEG), :]], axis=0).astype(bf16)
            sc = jnp.where(mask, sc * (DH ** -0.5), NEG)
            mx = jnp.max(sc, axis=1, keepdims=True)
            e = jnp.exp(sc - mx)
            den = jnp.sum(e, axis=1, keepdims=True)
            inv = pl.reciprocal(den, approx=True)
            inv = inv * (2.0 - den * inv)
            o = _dot(e.astype(bf16), va) * inv
            q_r[h][pl.ds(ra_, SEG), :] = o[MEM:]
            o_mem[h] = o[:MEM]

        def wo(h):
            lo = jnp.concatenate([o_mem.pop(h), q_r[h][pl.ds(rw_, TOK), :]],
                                 axis=0).astype(bf16)
            r = _dot(lo, _unpack(wo_b[pl.ds(h * DH // 2, DH // 2), :]))
            total[0] = r if total[0] is None else total[0] + r

        npair = H // 2
        for t in range(npair + LAG_WO):
            if 0 <= t - LAG_QK < npair:
                qk(2 * (t - LAG_QK))
                qk(2 * (t - LAG_QK) + 1)
            if 0 <= t - LAG_PV < npair:
                pv(2 * (t - LAG_PV))
                pv(2 * (t - LAG_PV) + 1)
            if t < npair:
                qkv(2 * t)
                qkv(2 * t + 1)
            if t == FILL_AT:
                filler(0)
            if 0 <= t - LAG_WO < npair:
                wo(2 * (t - LAG_WO))
                wo(2 * (t - LAG_WO) + 1)
        filler(1)

        a = total[0]
        hbuf[pl.ds(pl.multiple_of(TOK * s, 8), TOK), :] += a[MEM:]
        return a[:MEM], wrap(rp + TOK), wrap(ra + SEG), wrap(rw + TOK)

    def steps(i, carry):
        toks = [load_tok(i * UNROLL + k) for k in range(UNROLL)]
        for k in range(UNROLL):
            carry = step(i * UNROLL + k, carry, toks[k])
        return carry

    lax.fori_loop(
        0, NSEG // UNROLL, steps,
        (mem0_ref[...].astype(f32), jnp.int32(P0), jnp.int32(0), jnp.int32(0)))

    def tail(yall, t0, t1, acc):
        w2_copy.wait()
        w3_copy.wait()
        w4_copy.wait()

        def wo_batch(r0, n):
            rr = r0 % RING
            lo = jnp.concatenate(
                [q_r[h][pl.ds(rr, n), :].astype(bf16) for h in range(H)], axis=1)
            hbuf[pl.ds(r0, n), :] += _dot(lo, _unpack(wo_b[...]))

        def mixer_norm(r0, n):
            return _ln(_ln(hbuf[pl.ds(r0, n), :])).astype(bf16)

        def mixer_in(r0, u):
            for c in range(4):
                xg[c, pl.ds(HALO + r0, u.shape[0]), :] = _gelu(_dot(u, _unpack(w1b[c])))

        def mixer_out(i):
            hs = None
            for c, off in enumerate((-1, 1, -2, 2)):
                win = xg[c, pl.ds(i * RB, RB + 2 * HALO), :]
                g = win[HALO + off:HALO + off + RB].astype(bf16)
                r = _dot(g, _unpack(w2b[pl.ds(c * C4 // 2, C4 // 2), :]))
                hs = r if hs is None else hs + r
            return hs

        def mixer_post(i, hs):
            r0 = i * RB
            hv = hbuf[pl.ds(r0, RB), :]
            x1 = _ln(hv) + hs
            yall[pl.ds(r0 // 2, RB // 2), :] = _pack(_ln(x1))
            hbuf[pl.ds(r0, RB), :] = hv + x1

        done = TOK * NSEG
        split = 3 * RING
        first = 4 * TOK * (NSEG // 4 - 1)
        u = mixer_norm(first, done - first)
        wo_batch(done, split - done)
        mixer_in(first, u)
        u = mixer_norm(done, split - done)
        wo_batch(split, S - split)
        mixer_in(done, u)
        hs = {0: mixer_out(0), 1: mixer_out(1)}
        u = mixer_norm(split, S - split)
        hs[2] = mixer_out(2)
        mixer_post(0, hs.pop(0))
        mixer_in(split, u)
        mixer_post(1, hs.pop(1))
        hs[3] = mixer_out(3)
        mixer_post(2, hs.pop(2))
        hs[4] = mixer_out(4)
        for i in range(5, S // RB):
            hs[i] = mixer_out(i)
            mixer_post(i - 2, hs.pop(i - 2))
        mixer_post(S // RB - 2, hs.pop(S // RB - 2))
        mixer_post(S // RB - 1, hs.pop(S // RB - 1))

        ts = (t0, t1)
        nc = F // FC

        def mlp_block(i, carry):
            rows = pl.ds(pl.multiple_of(i * RB, RB), RB)

            def up(c):
                y = _unpack(yall[pl.ds(pl.multiple_of(i * (RB // 2), RB // 2), RB // 2), :])
                r = _dot(y, _unpack(w3b[:, c * FC:(c + 1) * FC]))
                ts[c % 2][...] = _pack(_gelu(r))

            def down(c):
                w = _unpack(w4b[c * FC // 2:(c + 1) * FC // 2, :])
                if c == nc - 1:
                    hb = RB // 2
                    rs = [_dot(_unpack(ts[c % 2][k * hb // 2:(k + 1) * hb // 2, :]), w)
                          for k in range(2)]
                    for k in range(2):
                        half = pl.ds(pl.multiple_of(i * RB + k * hb, hb), hb)
                        xs[half, :] = (acc[k * hb:(k + 1) * hb, :] + rs[k]).astype(bf16)
                        out_copy(2 * i + k).start()
                    return
                r = _dot(_unpack(ts[c % 2][...]), w)
                if c == 0:
                    acc[...] = hbuf[rows, :] + r
                else:
                    acc[...] += r

            up(0)
            for c in range(nc):
                if c + 1 < nc:
                    up(c + 1)
                down(c)
            return carry

        lax.fori_loop(0, S // RB, mlp_block, 0)
        for i in range(2 * S // RB):
            out_copy(i).wait()

    pl.run_scoped(
        tail,
        pltpu.VMEM((S // 2, D), u32),
        pltpu.VMEM((RB // 2, FC), u32),
        pltpu.VMEM((RB // 2, FC), u32),
        pltpu.VMEM((RB, D), f32),
    )


@jax.jit
def pallas_sequential_preLN__memory_aug_recurrent_mem_tr__mixer_s_mlp__prompt_kernel(
    A_x: jax.Array,
    A_mem0: jax.Array,
    A_Wq: jax.Array,
    A_Wk: jax.Array,
    A_Wv: jax.Array,
    A_Wo: jax.Array,
    A_seg_len: jax.Array,
    B_x: jax.Array,
    B_w1: jax.Array,
    B_w2: jax.Array,
    B_w3: jax.Array,
    B_w4: jax.Array,
):
    del A_seg_len, B_x
    hbm = pl.BlockSpec(memory_space=pl.ANY)
    vmem = pl.BlockSpec(memory_space=pltpu.VMEM)
    scratch = [
        pltpu.VMEM((H, D // 2, DH), u32),
        pltpu.VMEM((H, D // 2, DH), u32),
        pltpu.VMEM((H, D // 2, DH), u32),
        pltpu.VMEM((H * DH // 2, D), u32),
        pltpu.VMEM((S, D), bf16),
        pltpu.VMEM((S, D), f32),
        pltpu.VMEM((4, S + 2 * HALO, C4), f32),
        pltpu.VMEM((2 * TOK, D), u32),
        pltpu.VMEM((4, D // 2, C4), u32),
        pltpu.VMEM((D // 2, D), u32),
        pltpu.VMEM((D // 2, F), u32),
        pltpu.VMEM((F // 2, D), u32),
        pltpu.SemaphoreType.DMA((NSEM,)),
    ] + [pltpu.VMEM((H // 8, RING, DH), f32)] * 24
    out = pl.pallas_call(
        _kernel,
        out_shape=jax.ShapeDtypeStruct((S, D), A_x.dtype),
        in_specs=[hbm, vmem] + [hbm] * 8,
        out_specs=hbm,
        scratch_shapes=scratch,
        compiler_params=pltpu.CompilerParams(vmem_limit_bytes=126 * 1024 * 1024),
    )(A_x.reshape(S, D), A_mem0.reshape(MEM, D),
      A_Wq.reshape(D // 2, 2 * H, DH), A_Wk.reshape(D // 2, 2 * H, DH),
      A_Wv.reshape(D // 2, 2 * H, DH),
      A_Wo.reshape(H * DH, D), B_w1, B_w2, B_w3, B_w4)
    return out.reshape(A_x.shape)
```

```python
import functools

import jax
import jax.numpy as jnp
from jax import lax
import jax.experimental.pallas as pl
import jax.experimental.pallas.tpu as pltpu

S = 2048
D = 1024
H = 32
DH = 128
MEM = 8
SEG = 32
F = 3584
NSEG = S // SEG
L = MEM + SEG
TOK = 24
P0 = S - TOK * NSEG
RING = 576
XP = (S - P0) // 12
C4 = D // 4
HALO = 8
RB = 256
FC = 512
EPS = 1e-5
NEG = -1000000000.0

LAG_QK, LAG_PV, LAG_WO = 2, 4, 6
FILL_AT = 18
UNROLL = 2

bf16 = jnp.bfloat16
f32 = jnp.float32
u32 = jnp.uint32

SEM_X0, SEM_X, SEM_WO, SEM_W1, SEM_W2, SEM_W3, SEM_W4, SEM_OUT, SEM_W = (
    0, 1, 5, 9, 13, 14, 15, 16, 32)
NSEM = SEM_W + 12


def _mult(i, n):
    return i if isinstance(i, int) else pl.multiple_of(i, n)


def _ln(x):
    m = jnp.mean(x, axis=-1, keepdims=True)
    d = x - m
    v = jnp.mean(d * d, axis=-1, keepdims=True)
    return d * lax.rsqrt(v + EPS)


def _gelu(x):
    return jax.nn.gelu(x, approximate=True)


def _pack(x):
    return pltpu.bitcast(x.astype(bf16), u32)


def _unpack(x):
    return pltpu.bitcast(x, bf16)


def _dot(a, b):
    return jnp.dot(a, b, preferred_element_type=f32)


def _kernel(x_hbm, mem0_ref, wq_hbm, wk_hbm, wv_hbm, wo_hbm, w1_hbm, w2_hbm,
            w3_hbm, w4_hbm, out_hbm,
            wq_s, wk_s, wv_s, wo_b, xs, hbuf, xg, ubuf,
            w1b, w2b, w3b, w4b, sems, *rings):
    w_hbm = (wq_hbm, wk_hbm, wv_hbm)
    w_s = (wq_s, wk_s, wv_s)
    ring = [[rings[m * 8 + h % 8].at[h // 8] for h in range(H)] for m in range(3)]
    q_r, k_r, v_r = ring

    x0_copy = pltpu.make_async_copy(x_hbm.at[pl.ds(0, P0)], xs.at[pl.ds(0, P0)],
                                    sems.at[SEM_X0])

    def x_copy(g):
        rows = pl.ds(_mult(P0 + g * 3 * XP, XP), 3 * XP)
        return pltpu.make_async_copy(x_hbm.at[rows], xs.at[rows], sems.at[SEM_X + g])

    def wo_copy(i):
        rows = pl.ds(_mult(i * 512, 512), 512)
        return pltpu.make_async_copy(wo_hbm.bitcast(u32).at[rows], wo_b.at[rows],
                                     sems.at[SEM_WO + i])

    def w1_copy(i):
        cols = pl.ds(_mult(i * C4, C4), C4)
        return pltpu.make_async_copy(w1_hbm.bitcast(u32).at[:, cols], w1b.at[i],
                                     sems.at[SEM_W1 + i])

    w2_copy = pltpu.make_async_copy(w2_hbm.bitcast(u32), w2b, sems.at[SEM_W2])
    w3_copy = pltpu.make_async_copy(w3_hbm.bitcast(u32), w3b, sems.at[SEM_W3])
    w4_copy = pltpu.make_async_copy(w4_hbm.bitcast(u32), w4b, sems.at[SEM_W4])

    def out_copy(i):
        rows = pl.ds(_mult(i * (RB // 2), RB // 2), RB // 2)
        return pltpu.make_async_copy(xs.at[rows], out_hbm.at[rows], sems.at[SEM_OUT + i])

    def prologue(stg0, stg1, stg2, lhs0):
        stg = (stg0, stg1, stg2)

        def start_chunk(g, m):
            src = w_hbm[m].bitcast(u32)
            dst = stg[m].reshape(D // 2, 8, DH)
            for par in range(2):
                pltpu.make_async_copy(
                    src.at[:, pl.ds(_mult(16 * par + 4 * g, 4), 4), :],
                    dst.at[:, pl.ds(4 * par, 4), :],
                    sems.at[SEM_W + 3 * g + m]).start()

        def wait_chunk(g, m):
            pltpu.make_async_copy(stg[m], stg[m], sems.at[SEM_W + 3 * g + m]).wait()

        def relayout(g, m, pair, i0, n):
            ev = stg[m][pl.ds(8 * i0 + pair, n, stride=8), :]
            od = stg[m][pl.ds(8 * i0 + 4 + pair, n, stride=8), :]
            h = 8 * g + 2 * pair
            w_s[m][h, pl.ds(i0, n), :] = (ev & jnp.uint32(0xFFFF)) | (od << 16)
            w_s[m][h + 1, pl.ds(i0, n), :] = (ev >> 16) | (od & jnp.uint32(0xFFFF0000))

        def norm_rows(r0, n, to_lhs0):
            xv = xs[pl.ds(r0, n), :].astype(f32)
            hbuf[pl.ds(r0, n), :] = xv
            xn = _ln(xv)
            if to_lhs0:
                lhs0[pl.ds(pl.multiple_of(r0 // 2, n // 2), n // 2), :] = _pack(xn)
            else:
                for c in range(4):
                    xg[c, pl.ds(HALO + r0, n), :] = xn[:, c * C4:(c + 1) * C4]

        x0_copy.start()
        start_chunk(0, 0)
        start_chunk(0, 1)
        x_copy(0).start()
        start_chunk(0, 2)
        w1_copy(0).start()
        zero = jnp.zeros((HALO, C4), f32)
        for c in range(4):
            xg[c, pl.ds(0, HALO), :] = zero
            xg[c, pl.ds(HALO + S, HALO), :] = zero
        x0_copy.wait()

        @pl.loop(0, P0 // 128)
        def _(i):
            norm_rows(pl.multiple_of(i * 128, 128), 128, True)

        wait_chunk(0, 0)

        @pl.loop(0, 4)
        def _(pair):
            for i0 in range(0, D // 2, 64):
                relayout(0, 0, pair, i0, 64)

        def stage(g, m):
            c = 3 * g + m
            m1 = (m + 1) % 3
            g1 = jnp.minimum(g + (1 if m == 2 else 0), 3)
            pieces = [(pair, i0) for i0 in range(0, D // 2, 8) for pair in range(4)]
            wait_at = 5
            span = 8 - wait_at
            cuts = [len(pieces) * k // span for k in range(span + 1)]
            rcuts = [XP // 16 * k // span * 16 for k in range(span + 1)]
            for j in range(8):
                if j >= wait_at:
                    k = j - wait_at
                    for pair, i0 in pieces[cuts[k]:cuts[k + 1]]:
                        relayout(g1, m1, pair, i0, 8)
                    norm_rows(pl.multiple_of(P0 + c * XP + rcuts[k], 16),
                              rcuts[k + 1] - rcuts[k], False)
                res = _dot(_unpack(lhs0[...]), _unpack(w_s[m][8 * g + j]))
                if j == wait_at - 1:
                    pl.when(c < 11)(functools.partial(wait_chunk, g1, m1))
                    if m == 0:
                        x_copy(g).wait()
                if j == 7:
                    @pl.when(g < 3)
                    def _():
                        start_chunk(g + 1, m)
                        if m == 0:
                            x_copy(g + 1).start()
                        if m == 2:
                            w1_copy(g + 1).start()
                    if m == 1:
                        wo_copy(g).start()
                rings[m * 8 + j][g, pl.ds(0, P0), :] = res

        @pl.loop(0, 4)
        def _(g):
            for m in range(3):
                stage(g, m)

    pl.run_scoped(
        prologue,
        pltpu.VMEM((8 * D // 2, DH), u32),
        pltpu.VMEM((8 * D // 2, DH), u32),
        pltpu.VMEM((8 * D // 2, DH), u32),
        pltpu.VMEM((P0 // 2, D), u32),
    )
    w2_copy.start()
    w3_copy.start()
    w4_copy.start()
    for i in range(4):
        wo_copy(i).wait()
    for i in range(4):
        w1_copy(i).wait()

    def wrap(r):
        return jnp.where(r >= RING, r - RING, r)

    def load_tok(s):
        rows = pl.ds(pl.multiple_of(HALO + P0 + TOK * s, 8), TOK)
        return jnp.concatenate([xg[c, rows, :] for c in range(4)], axis=1)

    def step(s, carry, tok, first_of_group):
        mem, rp, ra, rw = carry
        ri = lax.broadcasted_iota(jnp.int32, (L, L), 0)
        ci = lax.broadcasted_iota(jnp.int32, (L, L), 1)
        mask = (ri < MEM) | (ri >= ci)

        lhs = jnp.concatenate([mem, tok], axis=0).astype(bf16)
        rps = [pl.multiple_of(wrap(rp + 8 * i), 8) for i in range(3)]
        ra_ = pl.multiple_of(ra, SEG)
        rw_ = pl.multiple_of(rw, 8)

        col = s & 3
        rb = pl.multiple_of(jnp.maximum((s >> 2) - 1, 0) * (4 * TOK), 8)
        if first_of_group:
            ubuf[...] = _pack(_ln(_ln(hbuf[pl.ds(rb, 4 * TOK), :])))

        def filler(j):
            r = _dot(_unpack(ubuf[...]), _unpack(w1b[col, :, pl.ds(j * 128, 128)]))
            xg[col, pl.ds(HALO + rb, 4 * TOK), pl.ds(j * 128, 128)] = _gelu(r)

        mem_qkv = {}
        scores = {}
        o_mem = {}
        total = [None]

        def qkv(h):
            res = []
            for m in range(3):
                r = _dot(lhs, _unpack(w_s[m][h]))
                for i in range(3):
                    ring[m][h][pl.ds(rps[i], 8), :] = r[8 + 8 * i:16 + 8 * i]
                res.append(r[:MEM])
            mem_qkv[h] = res

        def qk(h):
            qm, km, vm = mem_qkv.pop(h)
            qa = jnp.concatenate([qm, q_r[h][pl.ds(ra_, SEG), :]], axis=0).astype(bf16)
            ka = jnp.concatenate([km, k_r[h][pl.ds(ra_, SEG), :]], axis=0).astype(bf16)
            sc = lax.dot_general(qa, ka, (((1,), (1,)), ((), ())),
                                 preferred_element_type=f32)
            scores[h] = (sc, vm)

        def pv(h):
            sc, vm = scores.pop(h)
            va = jnp.concatenate([vm, v_r[h][pl.ds(ra_, SEG), :]], axis=0).astype(bf16)
            sc = jnp.where(mask, sc * (DH ** -0.5), NEG)
            mx = jnp.max(sc, axis=1, keepdims=True)
            e = jnp.exp(sc - mx)
            den = jnp.sum(e, axis=1, keepdims=True)
            inv = pl.reciprocal(den, approx=True)
            inv = inv * (2.0 - den * inv)
            o = _dot(e.astype(bf16), va) * inv
            q_r[h][pl.ds(ra_, SEG), :] = o[MEM:]
            o_mem[h] = o[:MEM]

        def wo(h):
            lo = jnp.concatenate([o_mem.pop(h), q_r[h][pl.ds(rw_, TOK), :]],
                                 axis=0).astype(bf16)
            r = _dot(lo, _unpack(wo_b[pl.ds(h * DH // 2, DH // 2), :]))
            total[0] = r if total[0] is None else total[0] + r

        npair = H // 2
        for t in range(npair + LAG_WO):
            if 0 <= t - LAG_QK < npair:
                qk(2 * (t - LAG_QK))
                qk(2 * (t - LAG_QK) + 1)
            if 0 <= t - LAG_PV < npair:
                pv(2 * (t - LAG_PV))
                pv(2 * (t - LAG_PV) + 1)
            if t < npair:
                qkv(2 * t)
                qkv(2 * t + 1)
            if t == FILL_AT:
                filler(0)
            if 0 <= t - LAG_WO < npair:
                wo(2 * (t - LAG_WO))
                wo(2 * (t - LAG_WO) + 1)
        filler(1)

        a = total[0]
        hbuf[pl.ds(pl.multiple_of(TOK * s, 8), TOK), :] += a[MEM:]
        return a[:MEM], wrap(rp + TOK), wrap(ra + SEG), wrap(rw + TOK)

    def steps(i, carry):
        toks = [load_tok(i * UNROLL + k) for k in range(UNROLL)]
        for k in range(UNROLL):
            carry = step(i * UNROLL + k, carry, toks[k], k == 0)
        return carry

    lax.fori_loop(
        0, NSEG // UNROLL, steps,
        (mem0_ref[...].astype(f32), jnp.int32(P0), jnp.int32(0), jnp.int32(0)))

    def tail(yall, t0, t1, acc):
        w2_copy.wait()
        w3_copy.wait()
        w4_copy.wait()

        def wo_batch(r0, n):
            rr = r0 % RING
            lo = jnp.concatenate(
                [q_r[h][pl.ds(rr, n), :].astype(bf16) for h in range(H)], axis=1)
            hbuf[pl.ds(r0, n), :] += _dot(lo, _unpack(wo_b[...]))

        def mixer_norm(r0, n):
            return _ln(_ln(hbuf[pl.ds(r0, n), :])).astype(bf16)

        def mixer_in(r0, u):
            for c in range(4):
                xg[c, pl.ds(HALO + r0, u.shape[0]), :] = _gelu(_dot(u, _unpack(w1b[c])))

        def mixer_out(i):
            hs = None
            for c, off in enumerate((-1, 1, -2, 2)):
                win = xg[c, pl.ds(i * RB, RB + 2 * HALO), :]
                g = win[HALO + off:HALO + off + RB].astype(bf16)
                r = _dot(g, _unpack(w2b[pl.ds(c * C4 // 2, C4 // 2), :]))
                hs = r if hs is None else hs + r
            return hs

        def mixer_post(i, hs):
            r0 = i * RB
            hv = hbuf[pl.ds(r0, RB), :]
            x1 = _ln(hv) + hs
            yall[pl.ds(r0 // 2, RB // 2), :] = _pack(_ln(x1))
            hbuf[pl.ds(r0, RB), :] = hv + x1

        done = TOK * NSEG
        split = 3 * RING
        first = 4 * TOK * (NSEG // 4 - 1)
        u = mixer_norm(first, done - first)
        wo_batch(done, split - done)
        mixer_in(first, u)
        u = mixer_norm(done, split - done)
        wo_batch(split, S - split)
        mixer_in(done, u)
        hs = {0: mixer_out(0), 1: mixer_out(1)}
        u = mixer_norm(split, S - split)
        hs[2] = mixer_out(2)
        mixer_post(0, hs.pop(0))
        mixer_in(split, u)
        mixer_post(1, hs.pop(1))
        hs[3] = mixer_out(3)
        mixer_post(2, hs.pop(2))
        hs[4] = mixer_out(4)
        for i in range(5, S // RB):
            hs[i] = mixer_out(i)
            mixer_post(i - 2, hs.pop(i - 2))
        mixer_post(S // RB - 2, hs.pop(S // RB - 2))
        mixer_post(S // RB - 1, hs.pop(S // RB - 1))

        ts = (t0, t1)
        nc = F // FC

        def mlp_block(i, carry):
            rows = pl.ds(pl.multiple_of(i * RB, RB), RB)

            def up(c):
                y = _unpack(yall[pl.ds(pl.multiple_of(i * (RB // 2), RB // 2), RB // 2), :])
                r = _dot(y, _unpack(w3b[:, c * FC:(c + 1) * FC]))
                ts[c % 2][...] = _pack(_gelu(r))

            def down(c):
                w = _unpack(w4b[c * FC // 2:(c + 1) * FC // 2, :])
                if c == nc - 1:
                    hb = RB // 2
                    rs = [_dot(_unpack(ts[c % 2][k * hb // 2:(k + 1) * hb // 2, :]), w)
                          for k in range(2)]
                    for k in range(2):
                        half = pl.ds(pl.multiple_of(i * RB + k * hb, hb), hb)
                        xs[half, :] = (acc[k * hb:(k + 1) * hb, :] + rs[k]).astype(bf16)
                        out_copy(2 * i + k).start()
                    return
                r = _dot(_unpack(ts[c % 2][...]), w)
                if c == 0:
                    acc[...] = hbuf[rows, :] + r
                else:
                    acc[...] += r

            up(0)
            for c in range(nc):
                if c + 1 < nc:
                    up(c + 1)
                down(c)
            return carry

        lax.fori_loop(0, S // RB, mlp_block, 0)
        for i in range(2 * S // RB):
            out_copy(i).wait()

    pl.run_scoped(
        tail,
        pltpu.VMEM((S // 2, D), u32),
        pltpu.VMEM((RB // 2, FC), u32),
        pltpu.VMEM((RB // 2, FC), u32),
        pltpu.VMEM((RB, D), f32),
    )


@jax.jit
def pallas_sequential_preLN__memory_aug_recurrent_mem_tr__mixer_s_mlp__prompt_kernel(
    A_x: jax.Array,
    A_mem0: jax.Array,
    A_Wq: jax.Array,
    A_Wk: jax.Array,
    A_Wv: jax.Array,
    A_Wo: jax.Array,
    A_seg_len: jax.Array,
    B_x: jax.Array,
    B_w1: jax.Array,
    B_w2: jax.Array,
    B_w3: jax.Array,
    B_w4: jax.Array,
):
    del A_seg_len, B_x
    hbm = pl.BlockSpec(memory_space=pl.ANY)
    vmem = pl.BlockSpec(memory_space=pltpu.VMEM)
    scratch = [
        pltpu.VMEM((H, D // 2, DH), u32),
        pltpu.VMEM((H, D // 2, DH), u32),
        pltpu.VMEM((H, D // 2, DH), u32),
        pltpu.VMEM((H * DH // 2, D), u32),
        pltpu.VMEM((S, D), bf16),
        pltpu.VMEM((S, D), f32),
        pltpu.VMEM((4, S + 2 * HALO, C4), f32),
        pltpu.VMEM((2 * TOK, D), u32),
        pltpu.VMEM((4, D // 2, C4), u32),
        pltpu.VMEM((D // 2, D), u32),
        pltpu.VMEM((D // 2, F), u32),
        pltpu.VMEM((F // 2, D), u32),
        pltpu.SemaphoreType.DMA((NSEM,)),
    ] + [pltpu.VMEM((H // 8, RING, DH), f32)] * 24
    out = pl.pallas_call(
        _kernel,
        out_shape=jax.ShapeDtypeStruct((S, D), A_x.dtype),
        in_specs=[hbm, vmem] + [hbm] * 8,
        out_specs=hbm,
        scratch_shapes=scratch,
        compiler_params=pltpu.CompilerParams(vmem_limit_bytes=126 * 1024 * 1024),
    )(A_x.reshape(S, D), A_mem0.reshape(MEM, D),
      A_Wq.reshape(D // 2, 2 * H, DH), A_Wk.reshape(D // 2, 2 * H, DH),
      A_Wv.reshape(D // 2, 2 * H, DH),
      A_Wo.reshape(H * DH, D), B_w1, B_w2, B_w3, B_w4)
    return out.reshape(A_x.shape)
```
